```python
import jax
import jax.numpy as jnp

def _softmax(x, axis=-1):
    return jax.nn.softmax(x, axis=axis)

def _gelu(x):
    return jax.nn.gelu(x, approximate=True)

def _silu(x):
    return jax.nn.silu(x)

def _sigmoid(x):
    return jax.nn.sigmoid(x)

def _layernorm(x, axis=-1, eps=1e-05):
    m = jnp.mean(x, axis=axis, keepdims=True)
    v = jnp.var(x, axis=axis, keepdims=True)
    return (x - m) / jnp.sqrt(v + eps)

def _scatter_add(tgt, idx, src, axis=0):
    return tgt.at[idx].add(src)

def _segment_sum(src, seg, n):
    return jax.ops.segment_sum(src, seg, n)

class _Rng:

    def __init__(self, key):
        self._k = key

    def _next(self):
        self._k, sub = jax.random.split(self._k)
        return sub

    def normal(self, shape):
        return jax.random.normal(self._next(), shape, dtype=jnp.bfloat16)

    def randint(self, lo, hi, shape):
        return jax.random.randint(self._next(), shape, lo, hi, dtype=jnp.int32)

    def uniform(self, shape, lo=0.0, hi=1.0):
        return jax.random.uniform(self._next(), shape, jnp.bfloat16, lo, hi)

    def permutation(self, n):
        return jax.random.permutation(self._next(), n)
kernel_name = 'interleave_layers__memory_aug_recurrent_mem_tr__glu_gated_geglu__prompt'

def setup_inputs():
    _rng = _Rng(jax.random.key(int.from_bytes(__import__("os").urandom(4), "little")))
    _w = lambda a: (lambda t: t.astype(jnp.bfloat16) if jnp.issubdtype(t.dtype, jnp.floating) else t)(jnp.asarray(a))

    def _A_setup():
        B, S, Dm = (1, 2048, 1024)
        H, Dh = (32, 128)
        M, seg = (8, 32)
        seg = min(seg, S)
        S = S // seg * seg
        return {'x': _w((lambda *s: _rng.normal(s) * 0.05)(B, S, Dm)), 'mem0': _w((lambda *s: _rng.normal(s) * 0.05)(B, M, Dm)), 'Wq': _w((lambda *s: _rng.normal(s) * 0.05)(Dm, H, Dh) * Dm ** (-0.5)), 'Wk': _w((lambda *s: _rng.normal(s) * 0.05)(Dm, H, Dh) * Dm ** (-0.5)), 'Wv': _w((lambda *s: _rng.normal(s) * 0.05)(Dm, H, Dh) * Dm ** (-0.5)), 'Wo': _w((lambda *s: _rng.normal(s) * 0.05)(H, Dh, Dm) * (H * Dh) ** (-0.5)), 'seg_len': seg}
    _A_in = _A_setup()

    def _B_setup():
        B, S, Dm, Df = (1, 2048, 1024, 3584)
        return {'x': _w((lambda *s: _rng.normal(s) * 0.05)(B, S, Dm)), 'w_gate': _w((lambda *s: _rng.normal(s) * 0.05)(Dm, Df) * Dm ** (-0.5)), 'w_up': _w((lambda *s: _rng.normal(s) * 0.05)(Dm, Df) * Dm ** (-0.5)), 'w_down': _w((lambda *s: _rng.normal(s) * 0.05)(Df, Dm) * Df ** (-0.5))}
    _B_in = _B_setup()
    return {'A_x': _A_in['x'], 'A_mem0': _A_in['mem0'], 'A_Wq': _A_in['Wq'], 'A_Wk': _A_in['Wk'], 'A_Wv': _A_in['Wv'], 'A_Wo': _A_in['Wo'], 'A_seg_len': _A_in['seg_len'], 'B_x': _B_in['x'], 'B_w_gate': _B_in['w_gate'], 'B_w_up': _B_in['w_up'], 'B_w_down': _B_in['w_down']}

def reference(A_x, A_mem0, A_Wq, A_Wk, A_Wv, A_Wo, A_seg_len, B_x, B_w_gate, B_w_up, B_w_down):

    def _A_ref(x, mem0, Wq, Wk, Wv, Wo, seg_len):
        B, S, Dm = x.shape
        H, Dh = (Wq.shape[1], Wq.shape[2])
        M = mem0.shape[1]
        scale = Dh ** (-0.5)
        n_seg = S // seg_len
        L = M + seg_len
        idx = jnp.arange(L)
        mask = (idx[:, None] < M) | (idx[:, None] >= idx[None, :])
        mem = mem0
        outs = []
        for s in range(n_seg):
            xs = x[:, s * seg_len:(s + 1) * seg_len, :].copy()
            h = jnp.concatenate([mem, xs], axis=1)
            q = jnp.einsum('btd,dhe->bhte', h, Wq)
            k = jnp.einsum('btd,dhe->bhte', h, Wk)
            v = jnp.einsum('btd,dhe->bhte', h, Wv)
            scores = jnp.einsum('bhqe,bhke->bhqk', q, k) * scale
            scores = jnp.where(mask[None, None], scores, -1000000000.0)
            p = _softmax(scores, axis=-1)
            o = jnp.einsum('bhqk,bhke->bhqe', p, v)
            o = jnp.einsum('bhte,hed->btd', o, Wo)
            mem = o[:, :M, :].copy()
            outs.append(o[:, M:, :])
        return jnp.concatenate(outs, axis=1)

    def _B_ref(x, w_gate, w_up, w_down):
        g = jnp.einsum('bsd,df->bsf', x, w_gate)
        u = jnp.einsum('bsd,df->bsf', x, w_up)
        h = _gelu(g) * u
        return jnp.einsum('bsf,fd->bsd', h, w_down)
    x = A_x
    x = x + _A_ref(_layernorm(x, axis=-1), A_mem0, A_Wq, A_Wk, A_Wv, A_Wo, A_seg_len)
    x = x + _B_ref(_layernorm(x, axis=-1), B_w_gate, B_w_up, B_w_down)
    x = x + _A_ref(_layernorm(x, axis=-1), A_mem0, A_Wq, A_Wk, A_Wv, A_Wo, A_seg_len)
    x = x + _B_ref(_layernorm(x, axis=-1), B_w_gate, B_w_up, B_w_down)
    return x
```

```python
import functools

import jax
import jax.numpy as jnp
import numpy as np
import jax.experimental.pallas as pl
import jax.experimental.pallas.tpu as pltpu

F32 = jnp.float32
BF16 = jnp.bfloat16
U32 = jnp.uint32

LANES = 128
HEADS_PER_DOT = 2
FF_TILES = 2
OUT_TILES = 2
DOWN_TILES = 1
STAGE_D = 128
STAGE_SLOTS = 4
UP_LOOP_TILES = 4
DOWN_LOOP_TILES = 2
DBG_STEPS = 0


def _layernorm(x):
    m = jnp.mean(x, axis=-1, keepdims=True)
    c = x - m
    v = jnp.mean(c * c, axis=-1, keepdims=True)
    return c * jax.lax.rsqrt(v + 1e-5)


def _gelu(x):
    return jax.nn.gelu(x, approximate=True)


def _dot(a, b):
    return jnp.dot(a, b, preferred_element_type=F32)


def _dot_nt(a, b):
    return jax.lax.dot_general(a, b, (((1,), (1,)), ((), ())), preferred_element_type=F32)


def _cat(ref, lo, n, rows=None):
    if ref.dtype == BF16:
        ref = ref.bitcast(U32)
    rows = slice(None) if rows is None else slice(0, rows // 2)
    return jnp.concatenate(
        [pltpu.bitcast(ref[lo + j, rows, :], BF16) for j in range(n)], axis=1)


def _tile(x, j):
    return x[:, j * LANES:(j + 1) * LANES]


def _kernel(x_hbm, mem0_ref, wq_hbm, wk_hbm, wv_hbm, wo_hbm, wg_hbm, wu_hbm, wd_hbm,
            out_hbm,
            x_buf, out_buf, wqkv, wo, wg, wu, wd, stage,
            h_att, o_att, x2_buf, h_ffn, r_ffn, r_ffn_old, mid, bias2, bias1,
            stage_sem, up_sem, down_sem, sems, *, seg, n_seg, n_heads, dh):
    n_mem, dm = mem0_ref.shape
    nd = dm // LANES
    nf = wg.shape[0]
    m2 = 2 * n_mem
    scale = dh ** -0.5

    def seg_rows(s):
        return pl.ds(pl.multiple_of(s * seg, seg), seg)

    def column_copy(src, dst, j, sem):
        cols = pl.ds(pl.multiple_of(j * LANES, LANES), LANES)
        return pltpu.make_async_copy(src.at[:, cols], dst.at[j], sem)

    head_rows = 4 * seg
    cp_x_head = pltpu.make_async_copy(
        x_hbm.at[0:head_rows], x_buf.at[0:head_rows], sems.at[0])
    cp_x_tail = pltpu.make_async_copy(
        x_hbm.at[head_rows:], x_buf.at[head_rows:], sems.at[1])
    cp_wo = [column_copy(wo_hbm, wo, j, sems.at[2]) for j in range(nd)]

    def up_copies(c):
        return [column_copy(src, dst, c * UP_LOOP_TILES + i, up_sem.at[c])
                for i in range(UP_LOOP_TILES) for src, dst in ((wg_hbm, wg), (wu_hbm, wu))]

    def down_copy(j):
        return column_copy(wd_hbm, wd, j, down_sem.at[j])

    n_chunk = dm // STAGE_D
    stage_rows = STAGE_D * n_heads
    srcs = (wq_hbm, wk_hbm, wv_hbm)

    def stage_copy(w, c):
        slot = c % STAGE_SLOTS
        return pltpu.make_async_copy(
            srcs[w].at[pl.ds(pl.multiple_of(c * stage_rows, stage_rows), stage_rows), :],
            stage.at[slot], stage_sem.at[slot])

    ahead = STAGE_SLOTS - 1
    for c in range(ahead):
        stage_copy(0, c).start()
    cp_x_head.start()
    stage_u32 = stage.bitcast(U32)
    half = n_heads // 2
    for w in range(3):
        def relayout(c, carry, w=w):
            @pl.when(c + ahead < n_chunk)
            def _():
                stage_copy(w, c + ahead).start()

            if w < 2:
                @pl.when(c + ahead >= n_chunk)
                def _():
                    stage_copy(w + 1, c + ahead - n_chunk).start()
            else:
                @pl.when(c + ahead == n_chunk)
                def _():
                    for cp in cp_wo:
                        cp.start()
                    for c2 in range(nf // UP_LOOP_TILES):
                        for cp in up_copies(c2):
                            cp.start()
                    for j in range(nd):
                        down_copy(j).start()
                    cp_x_tail.start()

            stage_copy(w, c).wait()
            slot = c % STAGE_SLOTS
            d0 = pl.ds(pl.multiple_of(c * (STAGE_D // 2), STAGE_D // 2), STAGE_D // 2)
            for j in range(half):
                ev = stage_u32[slot, pl.ds(j, STAGE_D // 2, stride=2 * half), :]
                od = stage_u32[slot, pl.ds(half + j, STAGE_D // 2, stride=2 * half), :]
                wqkv[2 * j * 3 + w, d0, :] = (ev & U32(0xFFFF)) | (od << 16)
                wqkv[(2 * j + 1) * 3 + w, d0, :] = (ev >> 16) | (od & U32(0xFFFF0000))
            return carry
        jax.lax.fori_loop(0, n_chunk, relayout, 0)

    def make_bias(ref, second_from):
        ri = jax.lax.broadcasted_iota(jnp.int32, ref.shape, 0)
        ci = jax.lax.broadcasted_iota(jnp.int32, ref.shape, 1)

        def second(i):
            return ((i >= n_mem) & (i < m2)) | (i >= second_from)

        visible = (ri < m2) | (ci <= ri)
        ref[...] = jnp.where(second(ri) == second(ci),
                             jnp.where(visible, 0.0, -1e9), -jnp.inf).astype(F32)

    make_bias(bias2, m2 + seg)
    make_bias(bias1, m2 + seg)

    def put(ref, rows, x, lo=0):
        for j in range(x.shape[1] // LANES):
            ref[lo + j, rows, :] = _tile(x, j)

    def reset_mem():
        m0 = mem0_ref[...].astype(F32)
        put(h_att, slice(0, m2), jnp.concatenate([m0, m0], axis=0).astype(BF16))

    def ffn_norm(slot=None):
        rows = slice(None) if slot is None else seg_rows(slot)
        put(h_ffn, rows, _layernorm(r_ffn[rows, :]).astype(BF16))

    def ffn_up(lo, n):
        hf = _cat(h_ffn, 0, nd)
        y = _gelu(_dot(hf, _cat(wg, lo, n))) * _dot(hf, _cat(wu, lo, n))
        put(mid, slice(None), y.astype(BF16), lo)

    def ffn_down(lo, n, res_ref, store):
        cols = pl.ds(lo * LANES if isinstance(lo, int) else pl.multiple_of(lo * LANES, LANES),
                     n * LANES)
        store(cols, _dot(_cat(mid, 0, nf), _cat(wd, lo, n)) + res_ref[:, cols])

    def ffn_alone(store, first=False):
        def up(c, carry):
            if first:
                for cp in up_copies(c):
                    cp.wait()
            ffn_up(c * UP_LOOP_TILES, UP_LOOP_TILES)
            return carry

        def down(c, carry):
            if first:
                for i in range(DOWN_LOOP_TILES):
                    down_copy(c * DOWN_LOOP_TILES + i).wait()
            ffn_down(c * DOWN_LOOP_TILES, DOWN_LOOP_TILES, r_ffn, store)
            return carry

        ffn_norm()
        jax.lax.fori_loop(0, nf // UP_LOOP_TILES, up, 0)
        jax.lax.fori_loop(0, nd // DOWN_LOOP_TILES, down, 0)

    def attention(inputs, fill=lambda: None, before_out=lambda: None):
        n_rows = m2 + len(inputs) * seg
        bias_ref = bias2 if len(inputs) == 2 else bias1

        def norm():
            for i, (load, _, _) in enumerate(inputs):
                put(h_att, slice(m2 + i * seg, m2 + (i + 1) * seg),
                    _layernorm(load(slice(None))).astype(BF16))

        qkvs, probs = {}, {}

        def project(lo, hi):
            y = _dot(_cat(h_att, 0, nd, n_rows), _cat(wqkv, 3 * lo, 3 * (hi - lo))).astype(BF16)
            for h in range(lo, hi):
                qkvs[h] = [_tile(y, 3 * (h - lo) + i) for i in range(3)]

        def score(lo, hi):
            for h in range(lo, hi):
                bias = bias_ref[...]
                s = jnp.where(bias == 0.0, _dot_nt(qkvs[h][0], qkvs[h][1]) * scale, bias)
                p = jnp.exp(s - jnp.max(s, axis=-1, keepdims=True))
                probs[h] = (p.astype(BF16), 1.0 / jnp.sum(p, axis=-1, keepdims=True))

        def mix(lo, hi):
            for h in range(lo, hi):
                p, inv = probs.pop(h)
                o_att[h, 0:n_rows, :] = (_dot(p, qkvs.pop(h)[2]) * inv).astype(BF16)

        def project_out(lo, n):
            cols = slice(lo * LANES, (lo + n) * LANES)
            y = _dot(_cat(o_att, 0, n_heads, n_rows), _cat(wo, lo, n))
            mem = y[0:m2]
            if len(inputs) == 1:
                keep = jnp.concatenate(
                    [h_att[j, 0:m2, :] for j in range(lo, lo + n)], axis=1).astype(F32)
                row = jax.lax.broadcasted_iota(jnp.int32, mem.shape, 0)
                mem = jnp.where(row // n_mem == inputs[0][2], mem, keep)
            put(h_att, slice(0, m2), mem.astype(BF16), lo)
            for i, (load, slot, _) in enumerate(inputs):
                rows = seg_rows(slot) if not isinstance(slot, int) else slice(slot * seg, (slot + 1) * seg)
                r_ffn[rows, cols] = load(cols) + y[m2 + i * seg:m2 + (i + 1) * seg]

        def run():
            g = HEADS_PER_DOT
            n_grp = n_heads // g
            for i in range(n_grp + 2):
                if i < n_grp:
                    project(i * g, (i + 1) * g)
                else:
                    fill()
                if 0 <= i - 2:
                    mix((i - 2) * g, (i - 1) * g)
                if 0 <= i - 1 < n_grp:
                    score((i - 1) * g, i * g)
            fill()
            before_out()
            for j in range(0, nd, OUT_TILES):
                project_out(j, OUT_TILES)

        return norm, run

    def load_x(s):
        return lambda cols: x_buf[seg_rows(s), cols].astype(F32)

    def load_x2(s):
        return lambda cols: x2_buf[seg_rows(s % 2), cols]

    def store_step(s_x2, s_out):
        def store(cols, y):
            x2_buf[seg_rows(s_x2 % 2), cols] = y[0:seg]
            out_buf[seg_rows(s_out), cols] = y[seg:].astype(BF16)
        return store

    reset_mem()
    cp_x_head.wait()

    def first_layer_only(s, carry):
        def wait_wo():
            @pl.when(s == 0)
            def _():
                for cp in cp_wo:
                    cp.wait()

        norm, run = attention([(load_x(s), s, 0)], before_out=wait_wo)
        norm()
        run()
        return carry

    jax.lax.fori_loop(0, 2, first_layer_only, 0)

    def store_x2(cols, y):
        x2_buf[:, cols] = y

    ffn_alone(store_x2, first=True)
    norm, run = attention([(load_x(2), 0, 0), (load_x2(0), 1, 1)])
    norm()
    run()
    ffn_norm()
    cp_x_tail.wait()

    def step(t, carry):
        store = store_step(t - 1, t - 3)
        down = list(range(0, nd, DOWN_TILES))

        def fill():
            ffn_down(down.pop(0), DOWN_TILES, r_ffn_old, store)

        norm, run = attention([(load_x(t), 0, 0), (load_x2(t - 2), 1, 1)], fill)
        r_ffn_old[...] = r_ffn[...]
        norm()
        for j in range(0, nf, FF_TILES):
            ffn_up(j, FF_TILES)
        run()
        fill()
        ffn_norm()
        while down:
            fill()
        return carry

    jax.lax.fori_loop(3, DBG_STEPS or n_seg, step, 0)

    done = (n_seg - 3) * seg
    cp_out_head = pltpu.make_async_copy(out_buf.at[0:done], out_hbm.at[0:done], sems.at[3])
    cp_out_tail = pltpu.make_async_copy(out_buf.at[done:], out_hbm.at[done:], sems.at[4])
    cp_out_head.start()
    ffn_alone(store_step(n_seg - 1, n_seg - 3))

    make_bias(bias1, m2)

    def second_layer_only(i, carry):
        norm, run = attention([(load_x2(n_seg - 2 + i), i, 1)])
        norm()
        run()
        return carry

    jax.lax.fori_loop(0, 2, second_layer_only, 0)

    def store_out(cols, y):
        out_buf[(n_seg - 2) * seg:, cols] = y.astype(BF16)

    ffn_alone(store_out)
    cp_out_tail.start()
    cp_out_head.wait()
    cp_out_tail.wait()


@functools.partial(jax.jit, static_argnames=("A_seg_len",))
def pallas_interleave_layers__memory_aug_recurrent_mem_tr__glu_gated_geglu__prompt_kernel(
    A_x: jax.Array,
    A_mem0: jax.Array,
    A_Wq: jax.Array,
    A_Wk: jax.Array,
    A_Wv: jax.Array,
    A_Wo: jax.Array,
    A_seg_len: int,
    B_x: jax.Array,
    B_w_gate: jax.Array,
    B_w_up: jax.Array,
    B_w_down: jax.Array,
):
    del B_x
    batch, s, dm = A_x.shape
    assert batch == 1
    _, n_heads, dh = A_Wq.shape
    n_mem = A_mem0.shape[1]
    dff = B_w_gate.shape[1]
    seg = int(A_seg_len)
    n_seg = s // seg
    rows = 2 * (n_mem + seg)
    nd, nf = dm // LANES, dff // LANES
    assert dh == LANES

    hbm = pl.BlockSpec(memory_space=pl.ANY)
    out = pl.pallas_call(
        functools.partial(_kernel, seg=seg, n_seg=n_seg, n_heads=n_heads, dh=dh),
        out_shape=jax.ShapeDtypeStruct((s, dm), A_x.dtype),
        in_specs=[hbm, pl.BlockSpec(memory_space=pltpu.VMEM)] + [hbm] * 7,
        out_specs=hbm,
        scratch_shapes=[
            pltpu.VMEM((s, dm), BF16),
            pltpu.VMEM((s, dm), BF16),
            pltpu.VMEM((3 * n_heads, dm // 2, dh), U32),
            pltpu.VMEM((nd, n_heads * dh, LANES), BF16),
            pltpu.VMEM((nf, dm, LANES), BF16),
            pltpu.VMEM((nf, dm, LANES), BF16),
            pltpu.VMEM((nd, dff, LANES), BF16),
            pltpu.VMEM((STAGE_SLOTS, STAGE_D * n_heads, dh), BF16),
            pltpu.VMEM((nd, rows, LANES), BF16),
            pltpu.VMEM((n_heads, rows, dh), BF16),
            pltpu.VMEM((2 * seg, dm), F32),
            pltpu.VMEM((nd, 2 * seg, LANES), BF16),
            pltpu.VMEM((2 * seg, dm), F32),
            pltpu.VMEM((2 * seg, dm), F32),
            pltpu.VMEM((nf, 2 * seg, LANES), BF16),
            pltpu.VMEM((rows, rows), F32),
            pltpu.VMEM((rows - seg, rows - seg), F32),
            pltpu.SemaphoreType.DMA((STAGE_SLOTS,)),
            pltpu.SemaphoreType.DMA((nf // UP_LOOP_TILES,)),
            pltpu.SemaphoreType.DMA((nd,)),
            pltpu.SemaphoreType.DMA((5,)),
        ],
        compiler_params=pltpu.CompilerParams(vmem_limit_bytes=100 * 2**20),
    )(
        A_x.reshape(s, dm),
        A_mem0.reshape(n_mem, dm),
        A_Wq.reshape(dm * n_heads, dh),
        A_Wk.reshape(dm * n_heads, dh),
        A_Wv.reshape(dm * n_heads, dh),
        A_Wo.reshape(n_heads * dh, dm),
        B_w_gate,
        B_w_up,
        B_w_down,
    )
    return out.reshape(A_x.shape)
```

```python
import functools

import jax
import jax.numpy as jnp
import numpy as np
import jax.experimental.pallas as pl
import jax.experimental.pallas.tpu as pltpu

F32 = jnp.float32
BF16 = jnp.bfloat16
U32 = jnp.uint32

LANES = 128
HEADS_PER_DOT = 1
FF_TILES = 2
OUT_TILES = 2
DOWN_TILES = 1
FILL = (1, 1, 0, 0)
STAGE_D = 128
UP_EARLY = 1
STAGE_SLOTS = 4
UP_LOOP_TILES = 4
DBG_STEPS = 0


def _layernorm(x):
    m = jnp.mean(x, axis=-1, keepdims=True)
    c = x - m
    v = jnp.mean(c * c, axis=-1, keepdims=True)
    return c * jax.lax.rsqrt(v + 1e-5)


def _gelu(x):
    return jax.nn.gelu(x, approximate=True)


def _dot(a, b):
    return jnp.dot(a, b, preferred_element_type=F32)


def _dot_nt(a, b):
    return jax.lax.dot_general(a, b, (((1,), (1,)), ((), ())), preferred_element_type=F32)


def _cat(ref, lo, n, rows=None):
    if ref.dtype == BF16:
        ref = ref.bitcast(U32)
    rows = slice(None) if rows is None else slice(0, rows // 2)
    return jnp.concatenate(
        [pltpu.bitcast(ref[lo + j, rows, :], BF16) for j in range(n)], axis=1)


def _tile(x, j):
    return x[:, j * LANES:(j + 1) * LANES]


def _kernel(x_hbm, mem0_ref, wq_hbm, wk_hbm, wv_hbm, wo_hbm, wg_hbm, wu_hbm, wd_hbm,
            out_hbm,
            x_buf, out_buf, wqkv, wo, wg, wu, wd, stage,
            h_att, o_att, x1_buf, x2_buf, h_ffn, r_ffn, r_ffn_old, mid, bias2, bias1,
            stage_sem, up_sem, down_sem, sems, *, seg, n_seg, n_heads, dh):
    n_mem, dm = mem0_ref.shape
    nd = dm // LANES
    nf = wg.shape[0]
    m2 = 2 * n_mem
    scale = dh ** -0.5

    def seg_rows(s):
        return pl.ds(pl.multiple_of(s * seg, seg), seg)

    def column_copy(src, dst, j, sem):
        cols = pl.ds(pl.multiple_of(j * LANES, LANES), LANES)
        return pltpu.make_async_copy(src.at[:, cols], dst.at[j], sem)

    head_rows = 4 * seg
    cp_x_head = pltpu.make_async_copy(
        x_hbm.at[0:head_rows], x_buf.at[0:head_rows], sems.at[0])
    cp_x_tail = pltpu.make_async_copy(
        x_hbm.at[head_rows:], x_buf.at[head_rows:], sems.at[1])
    cp_wo = [column_copy(wo_hbm, wo, j, sems.at[2]) for j in range(nd)]

    def up_copies(c):
        return [column_copy(src, dst, c * UP_LOOP_TILES + i, up_sem.at[c])
                for i in range(UP_LOOP_TILES) for src, dst in ((wg_hbm, wg), (wu_hbm, wu))]

    def down_copy(j):
        return column_copy(wd_hbm, wd, j, down_sem.at[j])

    n_chunk = dm // STAGE_D
    stage_rows = STAGE_D * n_heads
    srcs = (wq_hbm, wk_hbm, wv_hbm)

    def stage_copy(w, c):
        slot = c % STAGE_SLOTS
        return pltpu.make_async_copy(
            srcs[w].at[pl.ds(pl.multiple_of(c * stage_rows, stage_rows), stage_rows), :],
            stage.at[slot], stage_sem.at[slot])

    ahead = STAGE_SLOTS - 1
    for c in range(ahead):
        stage_copy(0, c).start()
    cp_x_head.start()
    stage_u32 = stage.bitcast(U32)
    half = n_heads // 2
    for w in range(3):
        def relayout(c, carry, w=w):
            @pl.when(c + ahead < n_chunk)
            def _():
                stage_copy(w, c + ahead).start()

            if w < 2:
                @pl.when(c + ahead >= n_chunk)
                def _():
                    stage_copy(w + 1, c + ahead - n_chunk).start()
            else:
                @pl.when(c + ahead == n_chunk)
                def _():
                    for cp in cp_wo:
                        cp.start()

            stage_copy(w, c).wait()
            slot = c % STAGE_SLOTS
            d0 = pl.ds(pl.multiple_of(c * (STAGE_D // 2), STAGE_D // 2), STAGE_D // 2)
            for j in range(half):
                ev = stage_u32[slot, pl.ds(j, STAGE_D // 2, stride=2 * half), :]
                od = stage_u32[slot, pl.ds(half + j, STAGE_D // 2, stride=2 * half), :]
                wqkv[2 * j * 3 + w, d0, :] = (ev & U32(0xFFFF)) | (od << 16)
                wqkv[(2 * j + 1) * 3 + w, d0, :] = (ev >> 16) | (od & U32(0xFFFF0000))
            return carry
        jax.lax.fori_loop(0, n_chunk, relayout, 0)

    def make_bias(ref, second_from):
        ri = jax.lax.broadcasted_iota(jnp.int32, ref.shape, 0)
        ci = jax.lax.broadcasted_iota(jnp.int32, ref.shape, 1)

        def second(i):
            return ((i >= n_mem) & (i < m2)) | (i >= second_from)

        visible = (ri < m2) | (ci <= ri)
        ref[...] = jnp.where(second(ri) == second(ci),
                             jnp.where(visible, 0.0, -1e9), -jnp.inf).astype(F32)

    make_bias(bias2, m2 + seg)
    make_bias(bias1, m2 + seg)

    def put(ref, rows, x, lo=0):
        for j in range(x.shape[1] // LANES):
            ref[lo + j, rows, :] = _tile(x, j)

    def reset_mem():
        m0 = mem0_ref[...].astype(F32)
        put(h_att, slice(0, m2), jnp.concatenate([m0, m0], axis=0).astype(BF16))

    def ffn_norm():
        put(h_ffn, slice(None), _layernorm(r_ffn[...]).astype(BF16))

    def ffn_up(lo, n):
        hf = _cat(h_ffn, 0, nd)
        y = _gelu(_dot(hf, _cat(wg, lo, n))) * _dot(hf, _cat(wu, lo, n))
        put(mid, slice(None), y.astype(BF16), lo)

    def ffn_down(lo, n, res_ref, store):
        cols = pl.ds(lo * LANES if isinstance(lo, int) else pl.multiple_of(lo * LANES, LANES),
                     n * LANES)
        store(cols, _dot(_cat(mid, 0, nf), _cat(wd, lo, n)) + res_ref[:, cols])

    def ffn_first(store):
        def up(c, carry):
            for cp in up_copies(c):
                cp.wait()
            ffn_up(c * UP_LOOP_TILES, UP_LOOP_TILES)
            return carry

        def down(j, carry):
            down_copy(j).wait()
            ffn_down(j, 1, r_ffn, store)
            return carry

        ffn_norm()
        jax.lax.fori_loop(0, nf // UP_LOOP_TILES, up, 0)
        jax.lax.fori_loop(0, nd, down, 0)

    def ffn_with(inputs, res_ref, store, norm_next):
        down = list(range(0, nd, DOWN_TILES))

        def fill(i):
            for _ in range(FILL[i]):
                ffn_down(down.pop(0), DOWN_TILES, res_ref, store)

        if inputs:
            norm, run = attention(inputs, fill)
            norm()
        for j in range(0, nf, FF_TILES):
            ffn_up(j, FF_TILES)
        if inputs:
            run()
        if norm_next:
            ffn_norm()
        while down:
            ffn_down(down.pop(0), DOWN_TILES, res_ref, store)

    def attention(inputs, fill=lambda i: None, before_out=lambda: None):
        n_rows = m2 + len(inputs) * seg
        bias_ref = bias2 if len(inputs) == 2 else bias1

        def norm():
            for i, (load, _, _) in enumerate(inputs):
                put(h_att, slice(m2 + i * seg, m2 + (i + 1) * seg),
                    _layernorm(load(slice(None))).astype(BF16))

        qkvs, probs = {}, {}

        def project(lo, hi):
            y = _dot(_cat(h_att, 0, nd, n_rows), _cat(wqkv, 3 * lo, 3 * (hi - lo))).astype(BF16)
            for h in range(lo, hi):
                qkvs[h] = [_tile(y, 3 * (h - lo) + i) for i in range(3)]

        def score(lo, hi):
            for h in range(lo, hi):
                bias = bias_ref[...]
                s = jnp.where(bias == 0.0, _dot_nt(qkvs[h][0], qkvs[h][1]) * scale, bias)
                p = jnp.exp(s - jnp.max(s, axis=-1, keepdims=True))
                probs[h] = (p.astype(BF16), 1.0 / jnp.sum(p, axis=-1, keepdims=True))

        def mix(lo, hi):
            for h in range(lo, hi):
                p, inv = probs.pop(h)
                o_att[h, 0:n_rows, :] = (_dot(p, qkvs.pop(h)[2]) * inv).astype(BF16)

        def project_out(lo, n):
            cols = slice(lo * LANES, (lo + n) * LANES)
            y = _dot(_cat(o_att, 0, n_heads, n_rows), _cat(wo, lo, n))
            mem = y[0:m2]
            if len(inputs) == 1:
                keep = jnp.concatenate(
                    [h_att[j, 0:m2, :] for j in range(lo, lo + n)], axis=1).astype(F32)
                row = jax.lax.broadcasted_iota(jnp.int32, mem.shape, 0)
                mem = jnp.where(row // n_mem == inputs[0][2], mem, keep)
            put(h_att, slice(0, m2), mem.astype(BF16), lo)
            for i, (load, slot, _) in enumerate(inputs):
                slot(cols, load(cols) + y[m2 + i * seg:m2 + (i + 1) * seg])

        def run():
            g = HEADS_PER_DOT
            n_grp = n_heads // g
            for i in range(n_grp + 2):
                if i < n_grp:
                    project(i * g, (i + 1) * g)
                else:
                    fill(i - n_grp)
                if 0 <= i - 2:
                    mix((i - 2) * g, (i - 1) * g)
                if 0 <= i - 1 < n_grp:
                    score((i - 1) * g, i * g)
            fill(2)
            before_out()
            for j in range(0, nd, OUT_TILES):
                project_out(j, OUT_TILES)

        return norm, run

    def load_x(s):
        return lambda cols: x_buf[seg_rows(s), cols].astype(F32)

    def load_x2(s):
        return lambda cols: x2_buf[seg_rows(s % 2), cols]

    def to_ffn(slot, ref=r_ffn):
        def store(cols, y):
            ref[seg_rows(slot), cols] = y
        return store

    def store_step(s_x2, s_out):
        def store(cols, y):
            x2_buf[seg_rows(s_x2 % 2), cols] = y[0:seg]
            out_buf[seg_rows(s_out), cols] = y[seg:].astype(BF16)
        return store

    reset_mem()
    cp_x_head.wait()

    def first_layer_only(s, carry):
        def wait_wo():
            @pl.when(s == 0)
            def _():
                for c in range(UP_EARLY):
                    for cp in up_copies(c):
                        cp.start()
                for cp in cp_wo:
                    cp.wait()
                for c in range(UP_EARLY, nf // UP_LOOP_TILES):
                    for cp in up_copies(c):
                        cp.start()

            @pl.when(s == 2)
            def _():
                for j in range(nd):
                    down_copy(j).start()

        norm, run = attention([(load_x(s), to_ffn(s, x1_buf), 0)], before_out=wait_wo)
        norm()
        run()
        return carry

    jax.lax.fori_loop(0, 3, first_layer_only, 0)

    def store_x2(cols, y):
        x2_buf[:, cols] = y

    r_ffn[...] = x1_buf[0:2 * seg, :]
    ffn_first(store_x2)
    cp_x_tail.start()
    r_ffn[0:seg, :] = x1_buf[2 * seg:, :]
    make_bias(bias1, m2)
    norm, run = attention([(load_x2(0), to_ffn(1), 1)])
    norm()
    run()
    ffn_norm()
    cp_x_tail.wait()

    def step(t, carry):
        r_ffn_old[...] = r_ffn[...]
        ffn_with([(load_x(t), to_ffn(0), 0), (load_x2(t - 2), to_ffn(1), 1)],
                 r_ffn_old, store_step(t - 1, t - 3), True)
        return carry

    jax.lax.fori_loop(3, DBG_STEPS or n_seg, step, 0)

    done = (n_seg - 3) * seg
    cp_out_head = pltpu.make_async_copy(out_buf.at[0:done], out_hbm.at[0:done], sems.at[3])
    cp_out_tail = pltpu.make_async_copy(out_buf.at[done:], out_hbm.at[done:], sems.at[4])
    cp_out_head.start()
    r_ffn_old[...] = r_ffn[...]
    ffn_with([(load_x2(n_seg - 2), to_ffn(0), 1)],
             r_ffn_old, store_step(n_seg - 1, n_seg - 3), False)
    norm, run = attention([(load_x2(n_seg - 1), to_ffn(1), 1)])
    norm()
    run()
    ffn_norm()

    def store_out(cols, y):
        out_buf[(n_seg - 2) * seg:, cols] = y.astype(BF16)

    ffn_with([], r_ffn, store_out, False)
    cp_out_tail.start()
    cp_out_head.wait()
    cp_out_tail.wait()


@functools.partial(jax.jit, static_argnames=("A_seg_len",))
def pallas_interleave_layers__memory_aug_recurrent_mem_tr__glu_gated_geglu__prompt_kernel(
    A_x: jax.Array,
    A_mem0: jax.Array,
    A_Wq: jax.Array,
    A_Wk: jax.Array,
    A_Wv: jax.Array,
    A_Wo: jax.Array,
    A_seg_len: int,
    B_x: jax.Array,
    B_w_gate: jax.Array,
    B_w_up: jax.Array,
    B_w_down: jax.Array,
):
    del B_x
    batch, s, dm = A_x.shape
    assert batch == 1
    _, n_heads, dh = A_Wq.shape
    n_mem = A_mem0.shape[1]
    dff = B_w_gate.shape[1]
    seg = int(A_seg_len)
    n_seg = s // seg
    rows = 2 * (n_mem + seg)
    nd, nf = dm // LANES, dff // LANES
    assert dh == LANES

    hbm = pl.BlockSpec(memory_space=pl.ANY)
    out = pl.pallas_call(
        functools.partial(_kernel, seg=seg, n_seg=n_seg, n_heads=n_heads, dh=dh),
        out_shape=jax.ShapeDtypeStruct((s, dm), A_x.dtype),
        in_specs=[hbm, pl.BlockSpec(memory_space=pltpu.VMEM)] + [hbm] * 7,
        out_specs=hbm,
        scratch_shapes=[
            pltpu.VMEM((s, dm), BF16),
            pltpu.VMEM((s, dm), BF16),
            pltpu.VMEM((3 * n_heads, dm // 2, dh), U32),
            pltpu.VMEM((nd, n_heads * dh, LANES), BF16),
            pltpu.VMEM((nf, dm, LANES), BF16),
            pltpu.VMEM((nf, dm, LANES), BF16),
            pltpu.VMEM((nd, dff, LANES), BF16),
            pltpu.VMEM((STAGE_SLOTS, STAGE_D * n_heads, dh), BF16),
            pltpu.VMEM((nd, rows, LANES), BF16),
            pltpu.VMEM((n_heads, rows, dh), BF16),
            pltpu.VMEM((3 * seg, dm), F32),
            pltpu.VMEM((2 * seg, dm), F32),
            pltpu.VMEM((nd, 2 * seg, LANES), BF16),
            pltpu.VMEM((2 * seg, dm), F32),
            pltpu.VMEM((2 * seg, dm), F32),
            pltpu.VMEM((nf, 2 * seg, LANES), BF16),
            pltpu.VMEM((rows, rows), F32),
            pltpu.VMEM((rows - seg, rows - seg), F32),
            pltpu.SemaphoreType.DMA((STAGE_SLOTS,)),
            pltpu.SemaphoreType.DMA((nf // UP_LOOP_TILES,)),
            pltpu.SemaphoreType.DMA((nd,)),
            pltpu.SemaphoreType.DMA((5,)),
        ],
        compiler_params=pltpu.CompilerParams(vmem_limit_bytes=100 * 2**20),
    )(
        A_x.reshape(s, dm),
        A_mem0.reshape(n_mem, dm),
        A_Wq.reshape(dm * n_heads, dh),
        A_Wk.reshape(dm * n_heads, dh),
        A_Wv.reshape(dm * n_heads, dh),
        A_Wo.reshape(n_heads * dh, dm),
        B_w_gate,
        B_w_up,
        B_w_down,
    )
    return out.reshape(A_x.shape)
```

```python
import functools

import jax
import jax.numpy as jnp
import numpy as np
import jax.experimental.pallas as pl
import jax.experimental.pallas.tpu as pltpu

F32 = jnp.float32
BF16 = jnp.bfloat16
U32 = jnp.uint32

LANES = 128
LOG2E = float(np.log2(np.e))
HEADS_PER_DOT = 1
FF_TILES = 2
OUT_TILES = 2
DOWN_TILES = 1
FILL = (1, 1, 0, 0)
STAGE_D = 128
UP_EARLY = 1
STAGE_SLOTS = 4
UP_LOOP_TILES = 4
DBG_STEPS = 0


def _layernorm(x):
    m = jnp.mean(x, axis=-1, keepdims=True)
    c = x - m
    v = jnp.mean(c * c, axis=-1, keepdims=True)
    return c * jax.lax.rsqrt(v + 1e-5)


def _gelu(x):
    return jax.nn.gelu(x, approximate=True)


def _reciprocal(x):
    r = pl.reciprocal(x, approx=True)
    return r * (2.0 - x * r)


def _dot(a, b):
    return jnp.dot(a, b, preferred_element_type=F32)


def _dot_nt(a, b):
    return jax.lax.dot_general(a, b, (((1,), (1,)), ((), ())), preferred_element_type=F32)


def _cat(ref, lo, n, rows=None):
    if ref.dtype == BF16:
        ref = ref.bitcast(U32)
    rows = slice(None) if rows is None else slice(0, rows // 2)
    return jnp.concatenate(
        [pltpu.bitcast(ref[lo + j, rows, :], BF16) for j in range(n)], axis=1)


def _tile(x, j):
    return x[:, j * LANES:(j + 1) * LANES]


def _kernel(x_hbm, mem0_ref, wq_hbm, wk_hbm, wv_hbm, wo_hbm, wg_hbm, wu_hbm, wd_hbm,
            out_hbm,
            x_buf, out_buf, wqkv, wo, wg, wu, wd, stage,
            h_att, o_att, x1_buf, x2_buf, h_ffn, r_ffn, r_ffn_old, mid, bias2, bias1,
            stage_sem, up_sem, down_sem, sems, *, seg, n_seg, n_heads, dh):
    n_mem, dm = mem0_ref.shape
    nd = dm // LANES
    nf = wg.shape[0]
    m2 = 2 * n_mem
    scale = dh ** -0.5

    def seg_rows(s):
        return pl.ds(pl.multiple_of(s * seg, seg), seg)

    def column_copy(src, dst, j, sem):
        cols = pl.ds(pl.multiple_of(j * LANES, LANES), LANES)
        return pltpu.make_async_copy(src.at[:, cols], dst.at[j], sem)

    head_rows = 4 * seg
    cp_x_head = pltpu.make_async_copy(
        x_hbm.at[0:head_rows], x_buf.at[0:head_rows], sems.at[0])
    cp_x_tail = pltpu.make_async_copy(
        x_hbm.at[head_rows:], x_buf.at[head_rows:], sems.at[1])
    cp_wo = [column_copy(wo_hbm, wo, j, sems.at[2]) for j in range(nd)]

    def up_copies(c):
        return [column_copy(src, dst, c * UP_LOOP_TILES + i, up_sem.at[c])
                for i in range(UP_LOOP_TILES) for src, dst in ((wg_hbm, wg), (wu_hbm, wu))]

    def down_copy(j):
        return column_copy(wd_hbm, wd, j, down_sem.at[j])

    n_chunk = dm // STAGE_D
    stage_rows = STAGE_D * n_heads
    srcs = (wq_hbm, wk_hbm, wv_hbm)

    def stage_copy(w, c):
        slot = c % STAGE_SLOTS
        return pltpu.make_async_copy(
            srcs[w].at[pl.ds(pl.multiple_of(c * stage_rows, stage_rows), stage_rows), :],
            stage.at[slot], stage_sem.at[slot])

    ahead = STAGE_SLOTS - 1
    for c in range(ahead):
        stage_copy(0, c).start()
    cp_x_head.start()
    stage_u32 = stage.bitcast(U32)
    half = n_heads // 2
    for w in range(3):
        def relayout(c, carry, w=w):
            @pl.when(c + ahead < n_chunk)
            def _():
                stage_copy(w, c + ahead).start()

            if w < 2:
                @pl.when(c + ahead >= n_chunk)
                def _():
                    stage_copy(w + 1, c + ahead - n_chunk).start()
            else:
                @pl.when(c + ahead == n_chunk)
                def _():
                    for cp in cp_wo:
                        cp.start()

            stage_copy(w, c).wait()
            slot = c % STAGE_SLOTS
            d0 = pl.ds(pl.multiple_of(c * (STAGE_D // 2), STAGE_D // 2), STAGE_D // 2)
            for j in range(half):
                ev = stage_u32[slot, pl.ds(j, STAGE_D // 2, stride=2 * half), :]
                od = stage_u32[slot, pl.ds(half + j, STAGE_D // 2, stride=2 * half), :]
                wqkv[2 * j * 3 + w, d0, :] = (ev & U32(0xFFFF)) | (od << 16)
                wqkv[(2 * j + 1) * 3 + w, d0, :] = (ev >> 16) | (od & U32(0xFFFF0000))
            return carry
        jax.lax.fori_loop(0, n_chunk, relayout, 0)

    def make_bias(ref, second_from):
        ri = jax.lax.broadcasted_iota(jnp.int32, ref.shape, 0)
        ci = jax.lax.broadcasted_iota(jnp.int32, ref.shape, 1)

        def second(i):
            return ((i >= n_mem) & (i < m2)) | (i >= second_from)

        visible = (ri < m2) | (ci <= ri)
        ref[...] = jnp.where(second(ri) == second(ci),
                             jnp.where(visible, 0.0, -1e9 / scale), -jnp.inf).astype(F32)

    make_bias(bias2, m2 + seg)
    make_bias(bias1, m2 + seg)

    def put(ref, rows, x, lo=0):
        for j in range(x.shape[1] // LANES):
            ref[lo + j, rows, :] = _tile(x, j)

    def reset_mem():
        m0 = mem0_ref[...].astype(F32)
        put(h_att, slice(0, m2), jnp.concatenate([m0, m0], axis=0).astype(BF16))

    def ffn_norm():
        put(h_ffn, slice(None), _layernorm(r_ffn[...]).astype(BF16))

    def ffn_up(lo, n):
        hf = _cat(h_ffn, 0, nd)
        y = _gelu(_dot(hf, _cat(wg, lo, n))) * _dot(hf, _cat(wu, lo, n))
        put(mid, slice(None), y.astype(BF16), lo)

    def ffn_down(lo, n, res_ref, store):
        cols = pl.ds(lo * LANES if isinstance(lo, int) else pl.multiple_of(lo * LANES, LANES),
                     n * LANES)
        store(cols, _dot(_cat(mid, 0, nf), _cat(wd, lo, n)) + res_ref[:, cols])

    def ffn_first(store):
        def up(c, carry):
            for cp in up_copies(c):
                cp.wait()
            ffn_up(c * UP_LOOP_TILES, UP_LOOP_TILES)
            return carry

        def down(j, carry):
            down_copy(j).wait()
            ffn_down(j, 1, r_ffn, store)
            return carry

        ffn_norm()
        jax.lax.fori_loop(0, nf // UP_LOOP_TILES, up, 0)
        jax.lax.fori_loop(0, nd, down, 0)

    def ffn_with(inputs, res_ref, store, norm_next):
        down = list(range(0, nd, DOWN_TILES))

        def fill(i):
            for _ in range(FILL[i]):
                ffn_down(down.pop(0), DOWN_TILES, res_ref, store)

        if inputs:
            norm, run = attention(inputs, fill)
            norm()
        for j in range(0, nf, FF_TILES):
            ffn_up(j, FF_TILES)
        if inputs:
            run()
        if norm_next:
            ffn_norm()
        while down:
            ffn_down(down.pop(0), DOWN_TILES, res_ref, store)

    def attention(inputs, fill=lambda i: None, before_out=lambda: None):
        n_rows = m2 + len(inputs) * seg
        bias_ref = bias2 if len(inputs) == 2 else bias1

        def norm():
            for i, (load, _, _) in enumerate(inputs):
                put(h_att, slice(m2 + i * seg, m2 + (i + 1) * seg),
                    _layernorm(load(slice(None))).astype(BF16))

        qkvs, probs = {}, {}

        def project(lo, hi):
            y = _dot(_cat(h_att, 0, nd, n_rows), _cat(wqkv, 3 * lo, 3 * (hi - lo))).astype(BF16)
            for h in range(lo, hi):
                qkvs[h] = [_tile(y, 3 * (h - lo) + i) for i in range(3)]

        def score(lo, hi):
            for h in range(lo, hi):
                bias = bias_ref[...]
                s = jnp.where(bias == 0.0, _dot_nt(qkvs[h][0], qkvs[h][1]), bias)
                p = jnp.exp2((s - jnp.max(s, axis=-1, keepdims=True)) * (scale * LOG2E))
                probs[h] = (p.astype(BF16), _reciprocal(jnp.sum(p, axis=-1, keepdims=True)))

        def mix(lo, hi):
            for h in range(lo, hi):
                p, inv = probs.pop(h)
                o_att[h, 0:n_rows, :] = (_dot(p, qkvs.pop(h)[2]) * inv).astype(BF16)

        def project_out(lo, n):
            cols = slice(lo * LANES, (lo + n) * LANES)
            y = _dot(_cat(o_att, 0, n_heads, n_rows), _cat(wo, lo, n))
            mem = y[0:m2]
            if len(inputs) == 1:
                keep = jnp.concatenate(
                    [h_att[j, 0:m2, :] for j in range(lo, lo + n)], axis=1).astype(F32)
                row = jax.lax.broadcasted_iota(jnp.int32, mem.shape, 0)
                mem = jnp.where(row // n_mem == inputs[0][2], mem, keep)
            put(h_att, slice(0, m2), mem.astype(BF16), lo)
            for i, (load, slot, _) in enumerate(inputs):
                slot(cols, load(cols) + y[m2 + i * seg:m2 + (i + 1) * seg])

        def run():
            g = HEADS_PER_DOT
            n_grp = n_heads // g
            for i in range(n_grp + 2):
                if i < n_grp:
                    project(i * g, (i + 1) * g)
                else:
                    fill(i - n_grp)
                if 0 <= i - 2:
                    mix((i - 2) * g, (i - 1) * g)
                if 0 <= i - 1 < n_grp:
                    score((i - 1) * g, i * g)
            fill(2)
            before_out()
            for j in range(0, nd, OUT_TILES):
                project_out(j, OUT_TILES)

        return norm, run

    def load_x(s):
        return lambda cols: x_buf[seg_rows(s), cols].astype(F32)

    def load_x2(s):
        return lambda cols: x2_buf[seg_rows(s % 2), cols]

    def to_ffn(slot, ref=r_ffn):
        def store(cols, y):
            ref[seg_rows(slot), cols] = y
        return store

    def store_step(s_x2, s_out):
        def store(cols, y):
            x2_buf[seg_rows(s_x2 % 2), cols] = y[0:seg]
            out_buf[seg_rows(s_out), cols] = y[seg:].astype(BF16)
        return store

    reset_mem()
    cp_x_head.wait()

    def first_layer_only(s, carry):
        def wait_wo():
            @pl.when(s == 0)
            def _():
                for c in range(UP_EARLY):
                    for cp in up_copies(c):
                        cp.start()
                for cp in cp_wo:
                    cp.wait()
                for c in range(UP_EARLY, nf // UP_LOOP_TILES):
                    for cp in up_copies(c):
                        cp.start()

            @pl.when(s == 1)
            def _():
                for j in range(nd):
                    down_copy(j).start()

        norm, run = attention([(load_x(s), to_ffn(s, x1_buf), 0)], before_out=wait_wo)
        norm()
        run()
        return carry

    jax.lax.fori_loop(0, 3, first_layer_only, 0)

    def store_x2(cols, y):
        x2_buf[:, cols] = y

    r_ffn[...] = x1_buf[0:2 * seg, :]
    ffn_first(store_x2)
    cp_x_tail.start()
    r_ffn[0:seg, :] = x1_buf[2 * seg:, :]
    make_bias(bias1, m2)
    norm, run = attention([(load_x2(0), to_ffn(1), 1)])
    norm()
    run()
    ffn_norm()
    cp_x_tail.wait()

    def step(t, carry):
        r_ffn_old[...] = r_ffn[...]
        ffn_with([(load_x(t), to_ffn(0), 0), (load_x2(t - 2), to_ffn(1), 1)],
                 r_ffn_old, store_step(t - 1, t - 3), True)
        return carry

    jax.lax.fori_loop(3, DBG_STEPS or n_seg, step, 0)

    done = (n_seg - 3) * seg
    cp_out_head = pltpu.make_async_copy(out_buf.at[0:done], out_hbm.at[0:done], sems.at[3])
    cp_out_tail = pltpu.make_async_copy(out_buf.at[done:], out_hbm.at[done:], sems.at[4])
    cp_out_head.start()
    r_ffn_old[...] = r_ffn[...]
    ffn_with([(load_x2(n_seg - 2), to_ffn(0), 1)],
             r_ffn_old, store_step(n_seg - 1, n_seg - 3), False)
    norm, run = attention([(load_x2(n_seg - 1), to_ffn(1), 1)])
    norm()
    run()
    ffn_norm()

    def store_out(cols, y):
        out_buf[(n_seg - 2) * seg:, cols] = y.astype(BF16)

    ffn_with([], r_ffn, store_out, False)
    cp_out_tail.start()
    cp_out_head.wait()
    cp_out_tail.wait()


@functools.partial(jax.jit, static_argnames=("A_seg_len",))
def pallas_interleave_layers__memory_aug_recurrent_mem_tr__glu_gated_geglu__prompt_kernel(
    A_x: jax.Array,
    A_mem0: jax.Array,
    A_Wq: jax.Array,
    A_Wk: jax.Array,
    A_Wv: jax.Array,
    A_Wo: jax.Array,
    A_seg_len: int,
    B_x: jax.Array,
    B_w_gate: jax.Array,
    B_w_up: jax.Array,
    B_w_down: jax.Array,
):
    del B_x
    batch, s, dm = A_x.shape
    assert batch == 1
    _, n_heads, dh = A_Wq.shape
    n_mem = A_mem0.shape[1]
    dff = B_w_gate.shape[1]
    seg = int(A_seg_len)
    n_seg = s // seg
    rows = 2 * (n_mem + seg)
    nd, nf = dm // LANES, dff // LANES
    assert dh == LANES

    hbm = pl.BlockSpec(memory_space=pl.ANY)
    out = pl.pallas_call(
        functools.partial(_kernel, seg=seg, n_seg=n_seg, n_heads=n_heads, dh=dh),
        out_shape=jax.ShapeDtypeStruct((s, dm), A_x.dtype),
        in_specs=[hbm, pl.BlockSpec(memory_space=pltpu.VMEM)] + [hbm] * 7,
        out_specs=hbm,
        scratch_shapes=[
            pltpu.VMEM((s, dm), BF16),
            pltpu.VMEM((s, dm), BF16),
            pltpu.VMEM((3 * n_heads, dm // 2, dh), U32),
            pltpu.VMEM((nd, n_heads * dh, LANES), BF16),
            pltpu.VMEM((nf, dm, LANES), BF16),
            pltpu.VMEM((nf, dm, LANES), BF16),
            pltpu.VMEM((nd, dff, LANES), BF16),
            pltpu.VMEM((STAGE_SLOTS, STAGE_D * n_heads, dh), BF16),
            pltpu.VMEM((nd, rows, LANES), BF16),
            pltpu.VMEM((n_heads, rows, dh), BF16),
            pltpu.VMEM((3 * seg, dm), F32),
            pltpu.VMEM((2 * seg, dm), F32),
            pltpu.VMEM((nd, 2 * seg, LANES), BF16),
            pltpu.VMEM((2 * seg, dm), F32),
            pltpu.VMEM((2 * seg, dm), F32),
            pltpu.VMEM((nf, 2 * seg, LANES), BF16),
            pltpu.VMEM((rows, rows), F32),
            pltpu.VMEM((rows - seg, rows - seg), F32),
            pltpu.SemaphoreType.DMA((STAGE_SLOTS,)),
            pltpu.SemaphoreType.DMA((nf // UP_LOOP_TILES,)),
            pltpu.SemaphoreType.DMA((nd,)),
            pltpu.SemaphoreType.DMA((5,)),
        ],
        compiler_params=pltpu.CompilerParams(vmem_limit_bytes=100 * 2**20),
    )(
        A_x.reshape(s, dm),
        A_mem0.reshape(n_mem, dm),
        A_Wq.reshape(dm * n_heads, dh),
        A_Wk.reshape(dm * n_heads, dh),
        A_Wv.reshape(dm * n_heads, dh),
        A_Wo.reshape(n_heads * dh, dm),
        B_w_gate,
        B_w_up,
        B_w_down,
    )
    return out.reshape(A_x.shape)
```

```python
import functools

import jax
import jax.numpy as jnp
import numpy as np
import jax.experimental.pallas as pl
import jax.experimental.pallas.tpu as pltpu

F32 = jnp.float32
BF16 = jnp.bfloat16
U32 = jnp.uint32

LANES = 128
LOG2E = float(np.log2(np.e))
HEADS_PER_DOT = 1
FF_TILES = 2
OUT_TILES = 2
DOWN_TILES = 1
FILL = (1, 1, 0, 0)
STAGE_D = 128
STAGE_SLOTS = 7
STAGE_PAD = 16
LAG = 2
N_EARLY = 7
V_HEADS = 16


def _layernorm(x):
    m = jnp.mean(x, axis=-1, keepdims=True)
    c = x - m
    v = jnp.mean(c * c, axis=-1, keepdims=True)
    return c * jax.lax.rsqrt(v + 1e-5)


def _gelu(x):
    return jax.nn.gelu(x, approximate=True)


def _reciprocal(x):
    r = pl.reciprocal(x, approx=True)
    return r * (2.0 - x * r)


def _dot(a, b):
    return jnp.dot(a, b, preferred_element_type=F32)


def _dot_nt(a, b):
    return jax.lax.dot_general(a, b, (((1,), (1,)), ((), ())), preferred_element_type=F32)


def _cat(ref, lo, n, rows=None):
    if ref.dtype == BF16:
        ref = ref.bitcast(U32)
    rows = slice(None) if rows is None else slice(rows.start // 2, rows.stop // 2)
    return jnp.concatenate(
        [pltpu.bitcast(ref[lo + j, rows, :], BF16) for j in range(n)], axis=1)


def _tile(x, j):
    return x[:, j * LANES:(j + 1) * LANES]


def _kernel(x_hbm, mem0_ref, wq_hbm, wk_hbm, wv_hbm, wo_hbm, wg_hbm, wu_hbm, wd_hbm,
            out_hbm,
            x_buf, out_buf, wq, wk, wv, wo, wg, wu, wd, stage,
            h_early, qkv_early, h_att, o_att, x1_buf, x2_buf, h_ffn, r_ffn, r_ffn_old, mid, bias2, bias1,
            stage_sem, sems, *, seg, n_seg, n_heads, dh):
    n_mem, dm = mem0_ref.shape
    nd = dm // LANES
    nf = wg.shape[0]
    m2 = 2 * n_mem
    scale = dh ** -0.5

    def seg_rows(s):
        return pl.ds(pl.multiple_of(s * seg, seg), seg)

    def column_copy(src, dst, j, sem):
        cols = slice(j * LANES, (j + 1) * LANES)
        return pltpu.make_async_copy(src.at[:, cols], dst.at[j], sem)

    head_rows = (LAG + 1 + N_EARLY) * seg
    cp_x_head = pltpu.make_async_copy(
        x_hbm.at[0:head_rows], x_buf.at[0:head_rows], sems.at[0])
    cp_x_tail = pltpu.make_async_copy(
        x_hbm.at[head_rows:], x_buf.at[head_rows:], sems.at[1])
    cp_wo = [column_copy(wo_hbm, wo, j, sems.at[2]) for j in range(nd)]

    cp_up = [column_copy(src, dst, j, sems.at[5])
             for j in range(nf) for src, dst in ((wg_hbm, wg), (wu_hbm, wu))]
    cp_down = [column_copy(wd_hbm, wd, j, sems.at[6]) for j in range(nd)]

    n_chunk = dm // STAGE_D
    stage_rows = STAGE_D * n_heads
    srcs = (wq_hbm, wk_hbm, wv_hbm)
    wqkv = (wq, wk, wv)

    def stage_copy(w, c):
        slot = (w * n_chunk + c) % STAGE_SLOTS
        return pltpu.make_async_copy(
            srcs[w].at[pl.ds(pl.multiple_of(c * stage_rows, stage_rows), stage_rows), :],
            stage.at[slot, STAGE_PAD:STAGE_PAD + stage_rows], stage_sem.at[slot])

    def put(ref, rows, x, lo=0):
        for j in range(x.shape[1] // LANES):
            ref[lo + j, rows, :] = _tile(x, j)

    def reset_mem(ref):
        m0 = mem0_ref[...].astype(F32)
        put(ref, slice(0, m2), jnp.concatenate([m0, m0], axis=0).astype(BF16))

    def early_rows(i):
        return pl.ds(pl.multiple_of(m2 + i * seg, m2), seg)

    def early_norm(i):
        s = jnp.where(i == 0, 0, i + LAG)
        put(h_early, early_rows(i), _layernorm(x_buf[seg_rows(s), :].astype(F32)).astype(BF16))

    def early_project(w, h):
        qkv_early[3 * h + w] = _dot(_cat(h_early, 0, nd), _cat(wqkv[w], h, 1)).astype(BF16)

    stage[:, 0:STAGE_PAD, :] = jnp.zeros((STAGE_SLOTS, STAGE_PAD, dh), BF16)
    stage[:, STAGE_PAD + stage_rows:, :] = jnp.zeros((STAGE_SLOTS, 6 * STAGE_PAD, dh), BF16)
    ahead = STAGE_SLOTS - 1
    stage_copy(0, 0).start()
    cp_x_head.start()
    for c in range(1, ahead):
        stage_copy(0, c).start()
    reset_mem(h_early)
    cp_x_head.wait()
    stage_u32 = stage.bitcast(U32)
    half = n_heads // 2
    sublane = jax.lax.broadcasted_iota(jnp.int32, (8, dh), 0)

    def gather_rows(slot, base):
        x = {c: stage_u32[slot, pl.ds(base + c, 8, stride=2 * half + 1), :]
             for c in range(-7, half)}
        for k in (1, 2, 4):
            x = {c: jnp.where((sublane & k) != 0, x[c - k], x[c])
                 for c in range(2 * k - 8, half)}
        return [x[j] for j in range(half)]

    for w in range(3):
        def relayout(c, carry, w=w):
            @pl.when(c + ahead < n_chunk)
            def _():
                stage_copy(w, c + ahead).start()

            if w < 2:
                @pl.when(c + ahead >= n_chunk)
                def _():
                    stage_copy(w + 1, c + ahead - n_chunk).start()
            else:
                @pl.when(c + ahead == n_chunk)
                def _():
                    for cp in cp_wo:
                        cp.start()

            stage_copy(w, c).wait()
            if w == 0:
                per = -(-(N_EARLY + 1) // n_chunk)
                for i in range(per):
                    early_norm(jnp.minimum(c * per + i, N_EARLY))
            per_chunk = n_heads // n_chunk
            slot = (w * n_chunk + c) % STAGE_SLOTS
            per_chunk = n_heads // n_chunk
            blocks = STAGE_D // 16
            for blk in range(blocks):
                if w > 0:
                    for i in range(per_chunk):
                        if i * blocks // per_chunk == blk:
                            early_project(w - 1, c * per_chunk + i)
                base = STAGE_PAD // 2 + blk * 16 * half
                evens = gather_rows(slot, base)
                odds = gather_rows(slot, base + half)
                d0 = pl.ds(pl.multiple_of(c * (STAGE_D // 2) + blk * 8, 8), 8)
                for j, (ev, od) in enumerate(zip(evens, odds)):
                    wqkv[w][2 * j, d0, :] = (ev & U32(0xFFFF)) | (od << 16)
                    wqkv[w][2 * j + 1, d0, :] = (ev >> 16) | (od & U32(0xFFFF0000))
            return carry
        jax.lax.fori_loop(0, n_chunk, relayout, 0)

    for cp in cp_up + cp_down:
        cp.start()

    def project_v(c, carry):
        for i in range(V_HEADS):
            early_project(2, c * V_HEADS + i)
        return carry

    jax.lax.fori_loop(0, n_heads // V_HEADS, project_v, 0)

    def make_bias(ref, second_from):
        ri = jax.lax.broadcasted_iota(jnp.int32, ref.shape, 0)
        ci = jax.lax.broadcasted_iota(jnp.int32, ref.shape, 1)

        def second(i):
            return ((i >= n_mem) & (i < m2)) | (i >= second_from)

        visible = (ri < m2) | (ci <= ri)
        ref[...] = jnp.where(second(ri) == second(ci),
                             jnp.where(visible, 0.0, -1e9 / scale), -jnp.inf).astype(F32)

    make_bias(bias2, m2 + seg)
    make_bias(bias1, m2 + seg)

    def ffn_norm():
        put(h_ffn, slice(None), _layernorm(r_ffn[...]).astype(BF16))

    def ffn_up(lo, n):
        hf = _cat(h_ffn, 0, nd)
        y = _gelu(_dot(hf, _cat(wg, lo, n))) * _dot(hf, _cat(wu, lo, n))
        put(mid, slice(None), y.astype(BF16), lo)

    def ffn_down(lo, n, res_ref, store):
        cols = slice(lo * LANES, (lo + n) * LANES)
        store(cols, _dot(_cat(mid, 0, nf), _cat(wd, lo, n)) + res_ref[:, cols])

    def ffn_with(inputs, res_ref, store, norm_next, early=None, before_down=lambda: None):
        down = list(range(0, nd, DOWN_TILES))

        def fill(i):
            for _ in range(FILL[i]):
                ffn_down(down.pop(0), DOWN_TILES, res_ref, store)

        if inputs:
            norm, run = attention(inputs, fill, early=early)
            norm()
        for j in range(0, nf, FF_TILES):
            ffn_up(j, FF_TILES)
        if inputs:
            run()
        if norm_next:
            ffn_norm()
        before_down()
        while down:
            ffn_down(down.pop(0), DOWN_TILES, res_ref, store)

    def attention(inputs, fill=lambda i: None, before_out=lambda: None, early=None):
        n_rows = m2 + len(inputs) * seg
        bias_ref = bias2 if len(inputs) == 2 else bias1

        def norm():
            for i, (load, _, _) in enumerate(inputs):
                if i == 0 and early is not None:
                    continue
                put(h_att, slice(m2 + i * seg, m2 + (i + 1) * seg),
                    _layernorm(load(slice(None))).astype(BF16))

        qkvs, probs = {}, {}

        def project(lo, hi):
            w = jnp.concatenate(
                [_cat(ref, h, 1) for h in range(lo, hi) for ref in wqkv], axis=1)
            if early is None:
                y = _dot(_cat(h_att, 0, nd, slice(0, n_rows)), w).astype(BF16)
            elif len(inputs) == 1:
                y = jnp.concatenate(
                    [qkv_early[j, 0:n_rows, :] for j in range(3 * lo, 3 * hi)], axis=1)
            else:
                lhs = jnp.concatenate([_cat(h_att, 0, nd, slice(0, m2)),
                                       _cat(h_att, 0, nd, slice(m2 + seg, n_rows))], axis=0)
                y = _dot(lhs, w).astype(BF16)
                done = jnp.concatenate(
                    [qkv_early[j, early_rows(early), :] for j in range(3 * lo, 3 * hi)], axis=1)
                y = jnp.concatenate([y[0:m2], done, y[m2:]], axis=0)
            for h in range(lo, hi):
                qkvs[h] = [_tile(y, 3 * (h - lo) + i) for i in range(3)]

        def score(lo, hi):
            for h in range(lo, hi):
                bias = bias_ref[...]
                s = jnp.where(bias == 0.0, _dot_nt(qkvs[h][0], qkvs[h][1]), bias)
                p = jnp.exp2((s - jnp.max(s, axis=-1, keepdims=True)) * (scale * LOG2E))
                probs[h] = (p.astype(BF16), _reciprocal(jnp.sum(p, axis=-1, keepdims=True)))

        def mix(lo, hi):
            for h in range(lo, hi):
                p, inv = probs.pop(h)
                o_att[h, 0:n_rows, :] = (_dot(p, qkvs.pop(h)[2]) * inv).astype(BF16)

        def project_out(lo, n):
            cols = slice(lo * LANES, (lo + n) * LANES)
            y = _dot(_cat(o_att, 0, n_heads, slice(0, n_rows)), _cat(wo, lo, n))
            mem = y[0:m2]
            if len(inputs) == 1:
                keep = jnp.concatenate(
                    [h_att[j, 0:m2, :] for j in range(lo, lo + n)], axis=1).astype(F32)
                row = jax.lax.broadcasted_iota(jnp.int32, mem.shape, 0)
                mem = jnp.where(row // n_mem == inputs[0][2], mem, keep)
            put(h_att, slice(0, m2), mem.astype(BF16), lo)
            for i, (load, slot, _) in enumerate(inputs):
                slot(cols, load(cols) + y[m2 + i * seg:m2 + (i + 1) * seg])

        def run():
            g = HEADS_PER_DOT
            n_grp = n_heads // g
            for i in range(n_grp + 2):
                if i < n_grp:
                    project(i * g, (i + 1) * g)
                else:
                    fill(i - n_grp)
                if 0 <= i - 2:
                    mix((i - 2) * g, (i - 1) * g)
                if 0 <= i - 1 < n_grp:
                    score((i - 1) * g, i * g)
            fill(2)
            before_out()
            for j in range(0, nd, OUT_TILES):
                project_out(j, OUT_TILES)

        return norm, run

    def load_x(s):
        return lambda cols: x_buf[seg_rows(s), cols].astype(F32)

    def load_x2(s):
        return lambda cols: x2_buf[seg_rows(s % 2), cols]

    def to_ffn(slot, ref=r_ffn):
        def store(cols, y):
            ref[seg_rows(slot), cols] = y
        return store

    def store_step(s_x2, s_out):
        def store(cols, y):
            x2_buf[seg_rows(s_x2 % 2), cols] = y[0:seg]
            out_buf[seg_rows(s_out), cols] = y[seg:].astype(BF16)
        return store

    def wait_wo():
        for cp in cp_wo:
            cp.wait()

    reset_mem(h_att)
    _, run = attention([(load_x(0), to_ffn(0, x1_buf), 0)], before_out=wait_wo, early=0)
    run()

    def first_layer_only(s, carry):
        norm, run = attention([(load_x(s), to_ffn(s, x1_buf), 0)])
        norm()
        run()
        return carry

    jax.lax.fori_loop(1, LAG + 1, first_layer_only, 0)

    def store_x2(cols, y):
        x2_buf[:, cols] = y

    def wait_down():
        for cp in cp_down:
            cp.wait()

    r_ffn[...] = x1_buf[0:2 * seg, :]
    ffn_norm()
    for cp in cp_up:
        cp.wait()
    ffn_with([], r_ffn, store_x2, False, before_down=wait_down)
    cp_x_tail.start()
    r_ffn[0:seg, :] = x1_buf[2 * seg:, :]
    make_bias(bias1, m2)
    norm, run = attention([(load_x2(0), to_ffn(1), 1)])
    norm()
    run()
    ffn_norm()

    def step(t, carry, early=False):
        r_ffn_old[...] = r_ffn[...]
        ffn_with([(load_x(t), to_ffn(0), 0), (load_x2(t - 2), to_ffn(1), 1)],
                 r_ffn_old, store_step(t - 1, t - 3), True, t - LAG if early else None)
        return carry

    first_full = LAG + 1 + N_EARLY
    jax.lax.fori_loop(LAG + 1, first_full, functools.partial(step, early=True), 0)
    cp_x_tail.wait()
    jax.lax.fori_loop(first_full, n_seg, step, 0)

    done = (n_seg - 3) * seg
    cp_out_head = pltpu.make_async_copy(out_buf.at[0:done], out_hbm.at[0:done], sems.at[3])
    cp_out_tail = pltpu.make_async_copy(out_buf.at[done:], out_hbm.at[done:], sems.at[4])
    cp_out_head.start()
    r_ffn_old[...] = r_ffn[...]
    ffn_with([(load_x2(n_seg - 2), to_ffn(0), 1)],
             r_ffn_old, store_step(n_seg - 1, n_seg - 3), False)
    norm, run = attention([(load_x2(n_seg - 1), to_ffn(1), 1)])
    norm()
    run()
    ffn_norm()

    def store_out(cols, y):
        out_buf[(n_seg - 2) * seg:, cols] = y.astype(BF16)

    ffn_with([], r_ffn, store_out, False)
    cp_out_tail.start()
    cp_out_head.wait()
    cp_out_tail.wait()


@functools.partial(jax.jit, static_argnames=("A_seg_len",))
def pallas_interleave_layers__memory_aug_recurrent_mem_tr__glu_gated_geglu__prompt_kernel(
    A_x: jax.Array,
    A_mem0: jax.Array,
    A_Wq: jax.Array,
    A_Wk: jax.Array,
    A_Wv: jax.Array,
    A_Wo: jax.Array,
    A_seg_len: int,
    B_x: jax.Array,
    B_w_gate: jax.Array,
    B_w_up: jax.Array,
    B_w_down: jax.Array,
):
    del B_x
    batch, s, dm = A_x.shape
    assert batch == 1
    _, n_heads, dh = A_Wq.shape
    n_mem = A_mem0.shape[1]
    dff = B_w_gate.shape[1]
    seg = int(A_seg_len)
    n_seg = s // seg
    rows = 2 * (n_mem + seg)
    early = 2 * n_mem + (1 + N_EARLY) * seg
    nd, nf = dm // LANES, dff // LANES
    assert dh == LANES

    hbm = pl.BlockSpec(memory_space=pl.ANY)
    out = pl.pallas_call(
        functools.partial(_kernel, seg=seg, n_seg=n_seg, n_heads=n_heads, dh=dh),
        out_shape=jax.ShapeDtypeStruct((s, dm), A_x.dtype),
        in_specs=[hbm, pl.BlockSpec(memory_space=pltpu.VMEM)] + [hbm] * 7,
        out_specs=hbm,
        scratch_shapes=[
            pltpu.VMEM((s, dm), BF16),
            pltpu.VMEM((s, dm), BF16),
            pltpu.VMEM((n_heads, dm // 2, dh), U32),
            pltpu.VMEM((n_heads, dm // 2, dh), U32),
            pltpu.VMEM((n_heads, dm // 2, dh), U32),
            pltpu.VMEM((nd, n_heads * dh, LANES), BF16),
            pltpu.VMEM((nf, dm, LANES), BF16),
            pltpu.VMEM((nf, dm, LANES), BF16),
            pltpu.VMEM((nd, dff, LANES), BF16),
            pltpu.VMEM((STAGE_SLOTS, STAGE_D * n_heads + 7 * STAGE_PAD, dh), BF16),
            pltpu.VMEM((nd, early, LANES), BF16),
            pltpu.VMEM((3 * n_heads, early, dh), BF16),
            pltpu.VMEM((nd, rows, LANES), BF16),
            pltpu.VMEM((n_heads, rows, dh), BF16),
            pltpu.VMEM((3 * seg, dm), F32),
            pltpu.VMEM((2 * seg, dm), F32),
            pltpu.VMEM((nd, 2 * seg, LANES), BF16),
            pltpu.VMEM((2 * seg, dm), F32),
            pltpu.VMEM((2 * seg, dm), F32),
            pltpu.VMEM((nf, 2 * seg, LANES), BF16),
            pltpu.VMEM((rows, rows), F32),
            pltpu.VMEM((rows - seg, rows - seg), F32),
            pltpu.SemaphoreType.DMA((STAGE_SLOTS,)),
            pltpu.SemaphoreType.DMA((7,)),
        ],
        compiler_params=pltpu.CompilerParams(vmem_limit_bytes=100 * 2**20),
    )(
        A_x.reshape(s, dm),
        A_mem0.reshape(n_mem, dm),
        A_Wq.reshape(dm * n_heads, dh),
        A_Wk.reshape(dm * n_heads, dh),
        A_Wv.reshape(dm * n_heads, dh),
        A_Wo.reshape(n_heads * dh, dm),
        B_w_gate,
        B_w_up,
        B_w_down,
    )
    return out.reshape(A_x.shape)
```

```python
import functools

import jax
import jax.numpy as jnp
import numpy as np
import jax.experimental.pallas as pl
import jax.experimental.pallas.tpu as pltpu

F32 = jnp.float32
BF16 = jnp.bfloat16
U32 = jnp.uint32

LANES = 128
LOG2E = float(np.log2(np.e))
HEADS_PER_DOT = 1
FF_TILES = 2
OUT_TILES = 2
DOWN_TILES = 1
FILL = (1, 1, 0, 0)
STAGE_D = 256
STAGE_SLOTS = 6
STAGE_PAD = 16
LAG = 2
N_EARLY = 9
UP_AT = 2
GATHER = 16
UNROLL = 1


def _layernorm(x):
    m = jnp.mean(x, axis=-1, keepdims=True)
    c = x - m
    v = jnp.mean(c * c, axis=-1, keepdims=True)
    return c * jax.lax.rsqrt(v + 1e-5)


def _gelu(x):
    return jax.nn.gelu(x, approximate=True)


def _reciprocal(x):
    r = pl.reciprocal(x, approx=True)
    return r * (2.0 - x * r)


def _dot(a, b):
    return jnp.dot(a, b, preferred_element_type=F32)


def _dot_nt(a, b):
    return jax.lax.dot_general(a, b, (((1,), (1,)), ((), ())), preferred_element_type=F32)


def _cat(ref, lo, n, rows=None):
    if ref.dtype == BF16:
        ref = ref.bitcast(U32)
    rows = slice(None) if rows is None else slice(rows.start // 2, rows.stop // 2)
    return jnp.concatenate(
        [pltpu.bitcast(ref[lo + j, rows, :], BF16) for j in range(n)], axis=1)


def _tile(x, j):
    return x[:, j * LANES:(j + 1) * LANES]


def _kernel(x_hbm, mem0_ref, wq_hbm, wk_hbm, wv_hbm, wo_hbm, wg_hbm, wu_hbm, wd_hbm,
            out_hbm,
            x_buf, out_buf, wq, wk, wv, wo, wg, wu, wd, stage,
            h_early, acc_early, qkv_early, h_att, o_att, x1_buf, x2_buf, h_ffn, r_ffn, r_ffn_old, mid, bias2, bias1,
            stage_sem, sems, *, seg, n_seg, n_heads, dh):
    n_mem, dm = mem0_ref.shape
    nd = dm // LANES
    nf = wg.shape[0]
    m2 = 2 * n_mem
    scale = dh ** -0.5

    def seg_rows(s):
        return pl.ds(pl.multiple_of(s * seg, seg), seg)

    def column_copy(src, dst, j, sem):
        cols = slice(j * LANES, (j + 1) * LANES)
        return pltpu.make_async_copy(src.at[:, cols], dst.at[j], sem)

    head_rows = (LAG + 1 + N_EARLY) * seg
    cp_x_head = pltpu.make_async_copy(
        x_hbm.at[0:head_rows], x_buf.at[0:head_rows], sems.at[0])
    cp_x_tail = pltpu.make_async_copy(
        x_hbm.at[head_rows:], x_buf.at[head_rows:], sems.at[1])
    cp_wo = [column_copy(wo_hbm, wo, j, sems.at[2]) for j in range(nd)]

    cp_up = [column_copy(src, dst, j, sems.at[5])
             for j in range(nf) for src, dst in ((wg_hbm, wg), (wu_hbm, wu))]
    cp_down = [column_copy(wd_hbm, wd, j, sems.at[6]) for j in range(nd)]

    n_chunk = dm // STAGE_D
    stage_rows = STAGE_D * n_heads
    srcs = (wq_hbm, wk_hbm, wv_hbm)
    wqkv = (wq, wk, wv)

    def stage_copy(w, c):
        slot = (w * n_chunk + c) % STAGE_SLOTS
        return pltpu.make_async_copy(
            srcs[w].at[pl.ds(pl.multiple_of(c * stage_rows, stage_rows), stage_rows), :],
            stage.at[slot, STAGE_PAD:STAGE_PAD + stage_rows], stage_sem.at[slot])

    def put(ref, rows, x, lo=0):
        for j in range(x.shape[1] // LANES):
            ref[lo + j, rows, :] = _tile(x, j)

    def reset_mem(ref):
        m0 = mem0_ref[...].astype(F32)
        put(ref, slice(0, m2), jnp.concatenate([m0, m0], axis=0).astype(BF16))

    def early_rows(i):
        return pl.ds(pl.multiple_of(m2 + i * seg, m2), seg)

    def early_norm(i, carry):
        s = jnp.where(i == 0, 0, i + LAG)
        put(h_early, early_rows(i), _layernorm(x_buf[seg_rows(s), :].astype(F32)).astype(BF16))
        return carry

    stage[:, 0:STAGE_PAD, :] = jnp.zeros((STAGE_SLOTS, STAGE_PAD, dh), BF16)
    stage[:, STAGE_PAD + stage_rows:, :] = jnp.zeros((STAGE_SLOTS, 6 * STAGE_PAD, dh), BF16)
    ahead = STAGE_SLOTS - 1
    cp_x_head.start()
    for i in range(ahead):
        stage_copy(i // n_chunk, i % n_chunk).start()
    reset_mem(h_early)
    acc_early[...] = jnp.zeros_like(acc_early)
    cp_x_head.wait()
    jax.lax.fori_loop(0, N_EARLY + 1, early_norm, 0)
    stage_u32 = stage.bitcast(U32)
    half = n_heads // 2
    sublane = jax.lax.broadcasted_iota(jnp.int32, (8, dh), 0)

    def gather_rows(slot, base):
        x = {c: stage_u32[slot, pl.ds(base + c, 8, stride=2 * half + 1), :]
             for c in range(-7, GATHER)}
        for k in (1, 2, 4):
            x = {c: jnp.where((sublane & k) != 0, x[c - k], x[c])
                 for c in range(2 * k - 8, GATHER)}
        return [x[j] for j in range(GATHER)]

    for w in range(3):
        def load_chunk(c, carry, w=w):
            nxt = w * n_chunk + c + ahead
            for w2 in range(w, 3):
                @pl.when(nxt // n_chunk == w2)
                def _():
                    stage_copy(w2, nxt - w2 * n_chunk).start()

            if w * n_chunk <= 3 * n_chunk - ahead < (w + 1) * n_chunk:
                @pl.when(nxt == 3 * n_chunk)
                def _():
                    for cp in cp_wo:
                        cp.start()

            if w == 2:
                @pl.when(c == UP_AT)
                def _():
                    for cp in cp_up:
                        cp.start()

            stage_copy(w, c).wait()
            slot = (w * n_chunk + c) % STAGE_SLOTS
            k_tiles = STAGE_D // LANES
            d0 = pl.multiple_of(c * (STAGE_D // 2), STAGE_D // 2)
            for j0 in range(0, half, GATHER):
                for blk in range(STAGE_D // 16):
                    base = STAGE_PAD // 2 + blk * 16 * half + j0
                    evens = gather_rows(slot, base)
                    odds = gather_rows(slot, base + half)
                    dst = pl.ds(pl.multiple_of(d0 + blk * 8, 8), 8)
                    for j, (ev, od) in enumerate(zip(evens, odds), j0):
                        wqkv[w][2 * j, dst, :] = (ev & U32(0xFFFF)) | (od << 16)
                        wqkv[w][2 * j + 1, dst, :] = (ev >> 16) | (od & U32(0xFFFF0000))
                for h in range(2 * j0, 2 * (j0 + GATHER)):
                    y = _dot(_cat(h_early, c * k_tiles, k_tiles),
                             pltpu.bitcast(wqkv[w][h, pl.ds(d0, STAGE_D // 2), :], BF16))
                    y = jnp.where(c == 0, y, acc_early[h] + y)
                    acc_early[h] = y
                    qkv_early[3 * h + w] = y.astype(BF16)
            return carry
        jax.lax.fori_loop(0, n_chunk, load_chunk, 0)

    def make_bias(ref, second_from):
        ri = jax.lax.broadcasted_iota(jnp.int32, ref.shape, 0)
        ci = jax.lax.broadcasted_iota(jnp.int32, ref.shape, 1)

        def second(i):
            return ((i >= n_mem) & (i < m2)) | (i >= second_from)

        visible = (ri < m2) | (ci <= ri)
        ref[...] = jnp.where(second(ri) == second(ci),
                             jnp.where(visible, 0.0, -1e9 / scale), -jnp.inf).astype(F32)

    make_bias(bias2, m2 + seg)
    make_bias(bias1, m2 + seg)

    def ffn_norm():
        put(h_ffn, slice(None), _layernorm(r_ffn[...]).astype(BF16))

    def ffn_up(lo, n):
        hf = _cat(h_ffn, 0, nd)
        y = _gelu(_dot(hf, _cat(wg, lo, n))) * _dot(hf, _cat(wu, lo, n))
        put(mid, slice(None), y.astype(BF16), lo)

    def ffn_down(lo, n, res_ref, store):
        cols = slice(lo * LANES, (lo + n) * LANES)
        store(cols, _dot(_cat(mid, 0, nf), _cat(wd, lo, n)) + res_ref[:, cols])

    def ffn_with(inputs, res_ref, store, norm_next, early=None, before_down=lambda: None):
        down = list(range(0, nd, DOWN_TILES))

        def fill(i):
            for _ in range(FILL[i]):
                ffn_down(down.pop(0), DOWN_TILES, res_ref, store)

        if inputs:
            norm, run = attention(inputs, fill, early=early)
            norm()
        for j in range(0, nf, FF_TILES):
            ffn_up(j, FF_TILES)
        if inputs:
            run()
        if norm_next:
            ffn_norm()
        before_down()
        while down:
            ffn_down(down.pop(0), DOWN_TILES, res_ref, store)

    def attention(inputs, fill=lambda i: None, before_out=lambda: None, early=None):
        n_rows = m2 + len(inputs) * seg
        bias_ref = bias2 if len(inputs) == 2 else bias1

        def norm():
            for i, (load, _, _) in enumerate(inputs):
                if i == 0 and early is not None:
                    continue
                put(h_att, slice(m2 + i * seg, m2 + (i + 1) * seg),
                    _layernorm(load(slice(None))).astype(BF16))

        qkvs, probs = {}, {}

        def project(lo, hi):
            w = jnp.concatenate(
                [_cat(ref, h, 1) for h in range(lo, hi) for ref in wqkv], axis=1)
            if early is None:
                y = _dot(_cat(h_att, 0, nd, slice(0, n_rows)), w).astype(BF16)
            elif len(inputs) == 1:
                y = jnp.concatenate(
                    [qkv_early[j, 0:n_rows, :] for j in range(3 * lo, 3 * hi)], axis=1)
            else:
                lhs = jnp.concatenate([_cat(h_att, 0, nd, slice(0, m2)),
                                       _cat(h_att, 0, nd, slice(m2 + seg, n_rows))], axis=0)
                y = _dot(lhs, w).astype(BF16)
                done = jnp.concatenate(
                    [qkv_early[j, early_rows(early), :] for j in range(3 * lo, 3 * hi)], axis=1)
                y = jnp.concatenate([y[0:m2], done, y[m2:]], axis=0)
            for h in range(lo, hi):
                qkvs[h] = [_tile(y, 3 * (h - lo) + i) for i in range(3)]

        def score(lo, hi):
            for h in range(lo, hi):
                bias = bias_ref[...]
                s = jnp.where(bias == 0.0, _dot_nt(qkvs[h][0], qkvs[h][1]), bias)
                p = jnp.exp2((s - jnp.max(s, axis=-1, keepdims=True)) * (scale * LOG2E))
                probs[h] = (p.astype(BF16), _reciprocal(jnp.sum(p, axis=-1, keepdims=True)))

        def mix(lo, hi):
            for h in range(lo, hi):
                p, inv = probs.pop(h)
                o_att[h, 0:n_rows, :] = (_dot(p, qkvs.pop(h)[2]) * inv).astype(BF16)

        def project_out(lo, n):
            cols = slice(lo * LANES, (lo + n) * LANES)
            y = _dot(_cat(o_att, 0, n_heads, slice(0, n_rows)), _cat(wo, lo, n))
            mem = y[0:m2]
            if len(inputs) == 1:
                keep = jnp.concatenate(
                    [h_att[j, 0:m2, :] for j in range(lo, lo + n)], axis=1).astype(F32)
                row = jax.lax.broadcasted_iota(jnp.int32, mem.shape, 0)
                mem = jnp.where(row // n_mem == inputs[0][2], mem, keep)
            put(h_att, slice(0, m2), mem.astype(BF16), lo)
            for i, (load, slot, _) in enumerate(inputs):
                slot(cols, load(cols) + y[m2 + i * seg:m2 + (i + 1) * seg])

        def run():
            g = HEADS_PER_DOT
            n_grp = n_heads // g
            for i in range(n_grp + 2):
                if i < n_grp:
                    project(i * g, (i + 1) * g)
                else:
                    fill(i - n_grp)
                if 0 <= i - 2:
                    mix((i - 2) * g, (i - 1) * g)
                if 0 <= i - 1 < n_grp:
                    score((i - 1) * g, i * g)
            fill(2)
            before_out()
            for j in range(0, nd, OUT_TILES):
                project_out(j, OUT_TILES)

        return norm, run

    def load_x(s):
        return lambda cols: x_buf[seg_rows(s), cols].astype(F32)

    def load_x2(s):
        return lambda cols: x2_buf[seg_rows(s % 2), cols]

    def to_ffn(slot, ref=r_ffn):
        def store(cols, y):
            ref[seg_rows(slot), cols] = y
        return store

    def store_step(s_x2, s_out):
        def store(cols, y):
            x2_buf[seg_rows(s_x2 % 2), cols] = y[0:seg]
            out_buf[seg_rows(s_out), cols] = y[seg:].astype(BF16)
        return store

    def wait_wo():
        for cp in cp_wo:
            cp.wait()

    reset_mem(h_att)
    _, run = attention([(load_x(0), to_ffn(0, x1_buf), 0)], before_out=wait_wo, early=0)
    run()

    for cp in cp_down:
        cp.start()
    def first_layer_only(s, carry):
        norm, run = attention([(load_x(s), to_ffn(s, x1_buf), 0)])
        norm()
        run()
        return carry

    jax.lax.fori_loop(1, LAG + 1, first_layer_only, 0)

    def store_x2(cols, y):
        x2_buf[:, cols] = y

    def wait_down():
        for cp in cp_down:
            cp.wait()

    r_ffn[...] = x1_buf[0:2 * seg, :]
    ffn_norm()
    for cp in cp_up:
        cp.wait()
    ffn_with([], r_ffn, store_x2, False, before_down=wait_down)
    cp_x_tail.start()
    r_ffn[0:seg, :] = x1_buf[2 * seg:, :]
    make_bias(bias1, m2)
    norm, run = attention([(load_x2(0), to_ffn(1), 1)])
    norm()
    run()
    ffn_norm()

    def step(t, carry, early=False):
        r_ffn_old[...] = r_ffn[...]
        ffn_with([(load_x(t), to_ffn(0), 0), (load_x2(t - 2), to_ffn(1), 1)],
                 r_ffn_old, store_step(t - 1, t - 3), True, t - LAG if early else None)
        return carry

    first_full = LAG + 1 + N_EARLY
    jax.lax.fori_loop(LAG + 1, first_full, functools.partial(step, early=True), 0)
    cp_x_tail.wait()
    jax.lax.fori_loop(first_full, n_seg, step, 0, unroll=UNROLL)

    done = (n_seg - 3) * seg
    cp_out_head = pltpu.make_async_copy(out_buf.at[0:done], out_hbm.at[0:done], sems.at[3])
    cp_out_tail = pltpu.make_async_copy(out_buf.at[done:], out_hbm.at[done:], sems.at[4])
    cp_out_head.start()
    r_ffn_old[...] = r_ffn[...]
    ffn_with([(load_x2(n_seg - 2), to_ffn(0), 1)],
             r_ffn_old, store_step(n_seg - 1, n_seg - 3), False)
    norm, run = attention([(load_x2(n_seg - 1), to_ffn(1), 1)])
    norm()
    run()
    ffn_norm()

    def store_out(cols, y):
        out_buf[(n_seg - 2) * seg:, cols] = y.astype(BF16)

    ffn_with([], r_ffn, store_out, False)
    cp_out_tail.start()
    cp_out_head.wait()
    cp_out_tail.wait()


@functools.partial(jax.jit, static_argnames=("A_seg_len",))
def pallas_interleave_layers__memory_aug_recurrent_mem_tr__glu_gated_geglu__prompt_kernel(
    A_x: jax.Array,
    A_mem0: jax.Array,
    A_Wq: jax.Array,
    A_Wk: jax.Array,
    A_Wv: jax.Array,
    A_Wo: jax.Array,
    A_seg_len: int,
    B_x: jax.Array,
    B_w_gate: jax.Array,
    B_w_up: jax.Array,
    B_w_down: jax.Array,
):
    del B_x
    batch, s, dm = A_x.shape
    assert batch == 1
    _, n_heads, dh = A_Wq.shape
    n_mem = A_mem0.shape[1]
    dff = B_w_gate.shape[1]
    seg = int(A_seg_len)
    n_seg = s // seg
    rows = 2 * (n_mem + seg)
    early = 2 * n_mem + (1 + N_EARLY) * seg
    nd, nf = dm // LANES, dff // LANES
    assert dh == LANES

    hbm = pl.BlockSpec(memory_space=pl.ANY)
    out = pl.pallas_call(
        functools.partial(_kernel, seg=seg, n_seg=n_seg, n_heads=n_heads, dh=dh),
        out_shape=jax.ShapeDtypeStruct((s, dm), A_x.dtype),
        in_specs=[hbm, pl.BlockSpec(memory_space=pltpu.VMEM)] + [hbm] * 7,
        out_specs=hbm,
        scratch_shapes=[
            pltpu.VMEM((s, dm), BF16),
            pltpu.VMEM((s, dm), BF16),
            pltpu.VMEM((n_heads, dm // 2, dh), U32),
            pltpu.VMEM((n_heads, dm // 2, dh), U32),
            pltpu.VMEM((n_heads, dm // 2, dh), U32),
            pltpu.VMEM((nd, n_heads * dh, LANES), BF16),
            pltpu.VMEM((nf, dm, LANES), BF16),
            pltpu.VMEM((nf, dm, LANES), BF16),
            pltpu.VMEM((nd, dff, LANES), BF16),
            pltpu.VMEM((STAGE_SLOTS, STAGE_D * n_heads + 7 * STAGE_PAD, dh), BF16),
            pltpu.VMEM((nd, early, LANES), BF16),
            pltpu.VMEM((n_heads, early, dh), F32),
            pltpu.VMEM((3 * n_heads, early, dh), BF16),
            pltpu.VMEM((nd, rows, LANES), BF16),
            pltpu.VMEM((n_heads, rows, dh), BF16),
            pltpu.VMEM((3 * seg, dm), F32),
            pltpu.VMEM((2 * seg, dm), F32),
            pltpu.VMEM((nd, 2 * seg, LANES), BF16),
            pltpu.VMEM((2 * seg, dm), F32),
            pltpu.VMEM((2 * seg, dm), F32),
            pltpu.VMEM((nf, 2 * seg, LANES), BF16),
            pltpu.VMEM((rows, rows), F32),
            pltpu.VMEM((rows - seg, rows - seg), F32),
            pltpu.SemaphoreType.DMA((STAGE_SLOTS,)),
            pltpu.SemaphoreType.DMA((7,)),
        ],
        compiler_params=pltpu.CompilerParams(vmem_limit_bytes=112 * 2**20),
    )(
        A_x.reshape(s, dm),
        A_mem0.reshape(n_mem, dm),
        A_Wq.reshape(dm * n_heads, dh),
        A_Wk.reshape(dm * n_heads, dh),
        A_Wv.reshape(dm * n_heads, dh),
        A_Wo.reshape(n_heads * dh, dm),
        B_w_gate,
        B_w_up,
        B_w_down,
    )
    return out.reshape(A_x.shape)
```

```python
import functools

import jax
import jax.numpy as jnp
import numpy as np
import jax.experimental.pallas as pl
import jax.experimental.pallas.tpu as pltpu

F32 = jnp.float32
BF16 = jnp.bfloat16
U32 = jnp.uint32

LANES = 128
LOG2E = float(np.log2(np.e))
HEADS_PER_DOT = 1
FF_TILES = 2
OUT_TILES = 2
DOWN_TILES = 1
FILL = (1, 1, 0, 0)
STAGE_D = 256
STAGE_SLOTS = 6
STAGE_PAD = 16
LAG = 2
N_EARLY = 10
UP_AT = 2
GATHER = 16
HEADS_SINGLE = 1
HEADS_FIRST = 16


def _layernorm(x):
    m = jnp.mean(x, axis=-1, keepdims=True)
    c = x - m
    v = jnp.mean(c * c, axis=-1, keepdims=True)
    return c * jax.lax.rsqrt(v + 1e-5)


def _gelu(x):
    return jax.nn.gelu(x, approximate=True)


def _reciprocal(x):
    r = pl.reciprocal(x, approx=True)
    return r * (2.0 - x * r)


def _dot(a, b):
    return jnp.dot(a, b, preferred_element_type=F32)


def _dot_nt(a, b):
    return jax.lax.dot_general(a, b, (((1,), (1,)), ((), ())), preferred_element_type=F32)


def _cat(ref, lo, n, rows=None):
    if ref.dtype == BF16:
        ref = ref.bitcast(U32)
    rows = slice(None) if rows is None else slice(rows.start // 2, rows.stop // 2)
    return jnp.concatenate(
        [pltpu.bitcast(ref[lo + j, rows, :], BF16) for j in range(n)], axis=1)


def _tile(x, j):
    return x[:, j * LANES:(j + 1) * LANES]


def _kernel(x_hbm, mem0_ref, wq_hbm, wk_hbm, wv_hbm, wo_hbm, wg_hbm, wu_hbm, wd_hbm,
            out_hbm,
            x_buf, out_buf, wq, wk, wv, wo, wg, wu, wd, stage,
            h_early, acc_early, qkv_early, h_att, o_att, x1_buf, x2_buf, h_ffn, r_ffn, r_ffn_old, mid, bias2, bias1,
            stage_sem, sems, *, seg, n_seg, n_heads, dh):
    n_mem, dm = mem0_ref.shape
    nd = dm // LANES
    nf = wg.shape[0]
    m2 = 2 * n_mem
    scale = dh ** -0.5

    def seg_rows(s):
        return pl.ds(pl.multiple_of(s * seg, seg), seg)

    def column_copy(src, dst, j, sem):
        cols = slice(j * LANES, (j + 1) * LANES)
        return pltpu.make_async_copy(src.at[:, cols], dst.at[j], sem)

    head_rows = (LAG + 1 + N_EARLY) * seg
    cp_x_head = pltpu.make_async_copy(
        x_hbm.at[0:head_rows], x_buf.at[0:head_rows], sems.at[0])
    cp_x_tail = pltpu.make_async_copy(
        x_hbm.at[head_rows:], x_buf.at[head_rows:], sems.at[1])
    cp_wo = [column_copy(wo_hbm, wo, j, sems.at[2]) for j in range(nd)]

    cp_up = [column_copy(src, dst, j, sems.at[5])
             for j in range(nf) for src, dst in ((wg_hbm, wg), (wu_hbm, wu))]
    cp_down = [column_copy(wd_hbm, wd, j, sems.at[6]) for j in range(nd)]

    n_chunk = dm // STAGE_D
    stage_rows = STAGE_D * n_heads
    srcs = (wq_hbm, wk_hbm, wv_hbm)
    wqkv = (wq, wk, wv)

    def stage_copy(w, c):
        slot = (w * n_chunk + c) % STAGE_SLOTS
        return pltpu.make_async_copy(
            srcs[w].at[pl.ds(pl.multiple_of(c * stage_rows, stage_rows), stage_rows), :],
            stage.at[slot, STAGE_PAD:STAGE_PAD + stage_rows], stage_sem.at[slot])

    def put(ref, rows, x, lo=0):
        for j in range(x.shape[1] // LANES):
            ref[lo + j, rows, :] = _tile(x, j)

    def reset_mem(ref):
        m0 = mem0_ref[...].astype(F32)
        put(ref, slice(0, m2), jnp.concatenate([m0, m0], axis=0).astype(BF16))

    def early_rows(i):
        return pl.ds(pl.multiple_of(m2 + i * seg, m2), seg)

    def early_norm(i, carry):
        s = jnp.where(i == 0, 0, i + LAG)
        put(h_early, early_rows(i), _layernorm(x_buf[seg_rows(s), :].astype(F32)).astype(BF16))
        return carry

    stage[:, 0:STAGE_PAD, :] = jnp.zeros((STAGE_SLOTS, STAGE_PAD, dh), BF16)
    stage[:, STAGE_PAD + stage_rows:, :] = jnp.zeros((STAGE_SLOTS, 6 * STAGE_PAD, dh), BF16)
    ahead = STAGE_SLOTS - 1
    cp_x_head.start()
    for i in range(ahead):
        stage_copy(i // n_chunk, i % n_chunk).start()
    reset_mem(h_early)
    acc_early[...] = jnp.zeros_like(acc_early)
    cp_x_head.wait()
    jax.lax.fori_loop(0, N_EARLY + 1, early_norm, 0)
    stage_u32 = stage.bitcast(U32)
    half = n_heads // 2
    sublane = jax.lax.broadcasted_iota(jnp.int32, (8, dh), 0)

    def gather_rows(slot, base):
        x = {c: stage_u32[slot, pl.ds(base + c, 8, stride=2 * half + 1), :]
             for c in range(-7, GATHER)}
        for k in (1, 2, 4):
            x = {c: jnp.where((sublane & k) != 0, x[c - k], x[c])
                 for c in range(2 * k - 8, GATHER)}
        return [x[j] for j in range(GATHER)]

    for w in range(3):
        def load_chunk(c, carry, w=w):
            nxt = w * n_chunk + c + ahead
            for w2 in range(w, 3):
                @pl.when(nxt // n_chunk == w2)
                def _():
                    stage_copy(w2, nxt - w2 * n_chunk).start()

            if w * n_chunk <= 3 * n_chunk - ahead < (w + 1) * n_chunk:
                @pl.when(nxt == 3 * n_chunk)
                def _():
                    for cp in cp_wo:
                        cp.start()

            if w == 2:
                @pl.when(c == UP_AT)
                def _():
                    for cp in cp_up:
                        cp.start()

            stage_copy(w, c).wait()
            slot = (w * n_chunk + c) % STAGE_SLOTS
            k_tiles = STAGE_D // LANES
            d0 = pl.multiple_of(c * (STAGE_D // 2), STAGE_D // 2)
            for j0 in range(0, half, GATHER):
                for blk in range(STAGE_D // 16):
                    base = STAGE_PAD // 2 + blk * 16 * half + j0
                    evens = gather_rows(slot, base)
                    odds = gather_rows(slot, base + half)
                    dst = pl.ds(pl.multiple_of(d0 + blk * 8, 8), 8)
                    for j, (ev, od) in enumerate(zip(evens, odds), j0):
                        wqkv[w][2 * j, dst, :] = (ev & U32(0xFFFF)) | (od << 16)
                        wqkv[w][2 * j + 1, dst, :] = (ev >> 16) | (od & U32(0xFFFF0000))
                for h in range(2 * j0, 2 * (j0 + GATHER)):
                    y = _dot(_cat(h_early, c * k_tiles, k_tiles),
                             pltpu.bitcast(wqkv[w][h, pl.ds(d0, STAGE_D // 2), :], BF16))
                    y = jnp.where(c == 0, y, acc_early[h] + y)
                    acc_early[h] = y
                    qkv_early[3 * h + w] = y.astype(BF16)
            return carry
        jax.lax.fori_loop(0, n_chunk, load_chunk, 0)

    def make_bias(ref, second_from):
        ri = jax.lax.broadcasted_iota(jnp.int32, ref.shape, 0)
        ci = jax.lax.broadcasted_iota(jnp.int32, ref.shape, 1)

        def second(i):
            return ((i >= n_mem) & (i < m2)) | (i >= second_from)

        visible = (ri < m2) | (ci <= ri)
        ref[...] = jnp.where(second(ri) == second(ci),
                             jnp.where(visible, 0.0, -1e9 / scale), -jnp.inf).astype(F32)

    make_bias(bias2, m2 + seg)
    make_bias(bias1, m2 + seg)

    def ffn_norm():
        put(h_ffn, slice(None), _layernorm(r_ffn[...]).astype(BF16))

    def ffn_up(lo, n):
        hf = _cat(h_ffn, 0, nd)
        y = _gelu(_dot(hf, _cat(wg, lo, n))) * _dot(hf, _cat(wu, lo, n))
        put(mid, slice(None), y.astype(BF16), lo)

    def ffn_down(lo, n, res_ref, store):
        cols = slice(lo * LANES, (lo + n) * LANES)
        store(cols, _dot(_cat(mid, 0, nf), _cat(wd, lo, n)) + res_ref[:, cols])

    def ffn_with(inputs, res_ref, store, norm_next, early=None, before_down=lambda: None):
        down = list(range(0, nd, DOWN_TILES))

        def fill(i):
            for _ in range(FILL[i]):
                ffn_down(down.pop(0), DOWN_TILES, res_ref, store)

        if inputs:
            norm, run = attention(inputs, fill, early=early)
            norm()
        for j in range(0, nf, FF_TILES):
            ffn_up(j, FF_TILES)
        if inputs:
            run()
        if norm_next:
            ffn_norm()
        before_down()
        while down:
            ffn_down(down.pop(0), DOWN_TILES, res_ref, store)

    def attention(inputs, fill=lambda i: None, before_out=lambda: None, early=None):
        n_rows = m2 + len(inputs) * seg
        bias_ref = bias2 if len(inputs) == 2 else bias1

        def norm():
            for i, (load, _, _) in enumerate(inputs):
                if i == 0 and early is not None:
                    continue
                put(h_att, slice(m2 + i * seg, m2 + (i + 1) * seg),
                    _layernorm(load(slice(None))).astype(BF16))

        qkvs, probs = {}, {}

        def project(lo, hi):
            w = jnp.concatenate(
                [_cat(ref, h, 1) for h in range(lo, hi) for ref in wqkv], axis=1)
            if early is None:
                y = _dot(_cat(h_att, 0, nd, slice(0, n_rows)), w).astype(BF16)
            elif len(inputs) == 1:
                y = jnp.concatenate(
                    [qkv_early[j, 0:n_rows, :] for j in range(3 * lo, 3 * hi)], axis=1)
            else:
                lhs = jnp.concatenate([_cat(h_att, 0, nd, slice(0, m2)),
                                       _cat(h_att, 0, nd, slice(m2 + seg, n_rows))], axis=0)
                y = _dot(lhs, w).astype(BF16)
                done = jnp.concatenate(
                    [qkv_early[j, early_rows(early), :] for j in range(3 * lo, 3 * hi)], axis=1)
                y = jnp.concatenate([y[0:m2], done, y[m2:]], axis=0)
            for h in range(lo, hi):
                qkvs[h] = [_tile(y, 3 * (h - lo) + i) for i in range(3)]

        def score(lo, hi):
            for h in range(lo, hi):
                bias = bias_ref[...]
                s = jnp.where(bias == 0.0, _dot_nt(qkvs[h][0], qkvs[h][1]), bias)
                p = jnp.exp2((s - jnp.max(s, axis=-1, keepdims=True)) * (scale * LOG2E))
                probs[h] = (p.astype(BF16), _reciprocal(jnp.sum(p, axis=-1, keepdims=True)))

        def mix(lo, hi):
            for h in range(lo, hi):
                p, inv = probs.pop(h)
                o_att[h, 0:n_rows, :] = (_dot(p, qkvs.pop(h)[2]) * inv).astype(BF16)

        def project_out(lo, n):
            cols = slice(lo * LANES, (lo + n) * LANES)
            y = _dot(_cat(o_att, 0, n_heads, slice(0, n_rows)), _cat(wo, lo, n))
            mem = y[0:m2]
            if len(inputs) == 1:
                keep = jnp.concatenate(
                    [h_att[j, 0:m2, :] for j in range(lo, lo + n)], axis=1).astype(F32)
                row = jax.lax.broadcasted_iota(jnp.int32, mem.shape, 0)
                mem = jnp.where(row // n_mem == inputs[0][2], mem, keep)
            put(h_att, slice(0, m2), mem.astype(BF16), lo)
            for i, (load, slot, _) in enumerate(inputs):
                slot(cols, load(cols) + y[m2 + i * seg:m2 + (i + 1) * seg])

        def run():
            if len(inputs) == 2:
                g = HEADS_PER_DOT
            else:
                g = HEADS_SINGLE if early is None else HEADS_FIRST
            n_grp = n_heads // g
            for i in range(n_grp + 2):
                if i < n_grp:
                    project(i * g, (i + 1) * g)
                else:
                    fill(i - n_grp)
                if 0 <= i - 2:
                    mix((i - 2) * g, (i - 1) * g)
                if 0 <= i - 1 < n_grp:
                    score((i - 1) * g, i * g)
            fill(2)
            before_out()
            for j in range(0, nd, OUT_TILES):
                project_out(j, OUT_TILES)

        return norm, run

    def load_x(s):
        return lambda cols: x_buf[seg_rows(s), cols].astype(F32)

    def load_x2(s):
        return lambda cols: x2_buf[seg_rows(s % 2), cols]

    def to_ffn(slot, ref=r_ffn):
        def store(cols, y):
            ref[seg_rows(slot), cols] = y
        return store

    def store_step(s_x2, s_out):
        def store(cols, y):
            x2_buf[seg_rows(s_x2 % 2), cols] = y[0:seg]
            out_buf[seg_rows(s_out), cols] = y[seg:].astype(BF16)
        return store

    def wait_wo():
        for cp in cp_wo:
            cp.wait()

    reset_mem(h_att)
    _, run = attention([(load_x(0), to_ffn(0, x1_buf), 0)], before_out=wait_wo, early=0)
    run()

    for cp in cp_down:
        cp.start()
    def first_layer_only(s, carry):
        norm, run = attention([(load_x(s), to_ffn(s, x1_buf), 0)])
        norm()
        run()
        return carry

    jax.lax.fori_loop(1, LAG + 1, first_layer_only, 0)

    def store_x2(cols, y):
        x2_buf[:, cols] = y

    def wait_down():
        for cp in cp_down:
            cp.wait()

    r_ffn[...] = x1_buf[0:2 * seg, :]
    ffn_norm()
    for cp in cp_up:
        cp.wait()
    ffn_with([], r_ffn, store_x2, False, before_down=wait_down)
    cp_x_tail.start()
    r_ffn[0:seg, :] = x1_buf[2 * seg:, :]
    make_bias(bias1, m2)
    norm, run = attention([(load_x2(0), to_ffn(1), 1)])
    norm()
    run()
    ffn_norm()

    def step(t, carry, early=False):
        r_ffn_old[...] = r_ffn[...]
        ffn_with([(load_x(t), to_ffn(0), 0), (load_x2(t - 2), to_ffn(1), 1)],
                 r_ffn_old, store_step(t - 1, t - 3), True, t - LAG if early else None)
        return carry

    first_full = LAG + 1 + N_EARLY
    jax.lax.fori_loop(LAG + 1, first_full, functools.partial(step, early=True), 0)
    cp_x_tail.wait()
    jax.lax.fori_loop(first_full, n_seg, step, 0)

    done = (n_seg - 3) * seg
    cp_out_head = pltpu.make_async_copy(out_buf.at[0:done], out_hbm.at[0:done], sems.at[3])
    cp_out_tail = pltpu.make_async_copy(out_buf.at[done:], out_hbm.at[done:], sems.at[4])
    cp_out_head.start()
    r_ffn_old[...] = r_ffn[...]
    ffn_with([(load_x2(n_seg - 2), to_ffn(0), 1)],
             r_ffn_old, store_step(n_seg - 1, n_seg - 3), False)
    norm, run = attention([(load_x2(n_seg - 1), to_ffn(1), 1)])
    norm()
    run()
    ffn_norm()

    def store_out(cols, y):
        out_buf[(n_seg - 2) * seg:, cols] = y.astype(BF16)

    ffn_with([], r_ffn, store_out, False)
    cp_out_tail.start()
    cp_out_head.wait()
    cp_out_tail.wait()


@functools.partial(jax.jit, static_argnames=("A_seg_len",))
def pallas_interleave_layers__memory_aug_recurrent_mem_tr__glu_gated_geglu__prompt_kernel(
    A_x: jax.Array,
    A_mem0: jax.Array,
    A_Wq: jax.Array,
    A_Wk: jax.Array,
    A_Wv: jax.Array,
    A_Wo: jax.Array,
    A_seg_len: int,
    B_x: jax.Array,
    B_w_gate: jax.Array,
    B_w_up: jax.Array,
    B_w_down: jax.Array,
):
    del B_x
    batch, s, dm = A_x.shape
    assert batch == 1
    _, n_heads, dh = A_Wq.shape
    n_mem = A_mem0.shape[1]
    dff = B_w_gate.shape[1]
    seg = int(A_seg_len)
    n_seg = s // seg
    rows = 2 * (n_mem + seg)
    early = 2 * n_mem + (1 + N_EARLY) * seg
    nd, nf = dm // LANES, dff // LANES
    assert dh == LANES

    hbm = pl.BlockSpec(memory_space=pl.ANY)
    out = pl.pallas_call(
        functools.partial(_kernel, seg=seg, n_seg=n_seg, n_heads=n_heads, dh=dh),
        out_shape=jax.ShapeDtypeStruct((s, dm), A_x.dtype),
        in_specs=[hbm, pl.BlockSpec(memory_space=pltpu.VMEM)] + [hbm] * 7,
        out_specs=hbm,
        scratch_shapes=[
            pltpu.VMEM((s, dm), BF16),
            pltpu.VMEM((s, dm), BF16),
            pltpu.VMEM((n_heads, dm // 2, dh), U32),
            pltpu.VMEM((n_heads, dm // 2, dh), U32),
            pltpu.VMEM((n_heads, dm // 2, dh), U32),
            pltpu.VMEM((nd, n_heads * dh, LANES), BF16),
            pltpu.VMEM((nf, dm, LANES), BF16),
            pltpu.VMEM((nf, dm, LANES), BF16),
            pltpu.VMEM((nd, dff, LANES), BF16),
            pltpu.VMEM((STAGE_SLOTS, STAGE_D * n_heads + 7 * STAGE_PAD, dh), BF16),
            pltpu.VMEM((nd, early, LANES), BF16),
            pltpu.VMEM((n_heads, early, dh), F32),
            pltpu.VMEM((3 * n_heads, early, dh), BF16),
            pltpu.VMEM((nd, rows, LANES), BF16),
            pltpu.VMEM((n_heads, rows, dh), BF16),
            pltpu.VMEM((3 * seg, dm), F32),
            pltpu.VMEM((2 * seg, dm), F32),
            pltpu.VMEM((nd, 2 * seg, LANES), BF16),
            pltpu.VMEM((2 * seg, dm), F32),
            pltpu.VMEM((2 * seg, dm), F32),
            pltpu.VMEM((nf, 2 * seg, LANES), BF16),
            pltpu.VMEM((rows, rows), F32),
            pltpu.VMEM((rows - seg, rows - seg), F32),
            pltpu.SemaphoreType.DMA((STAGE_SLOTS,)),
            pltpu.SemaphoreType.DMA((7,)),
        ],
        compiler_params=pltpu.CompilerParams(vmem_limit_bytes=112 * 2**20),
    )(
        A_x.reshape(s, dm),
        A_mem0.reshape(n_mem, dm),
        A_Wq.reshape(dm * n_heads, dh),
        A_Wk.reshape(dm * n_heads, dh),
        A_Wv.reshape(dm * n_heads, dh),
        A_Wo.reshape(n_heads * dh, dm),
        B_w_gate,
        B_w_up,
        B_w_down,
    )
    return out.reshape(A_x.shape)
```

```python
import functools

import jax
import jax.numpy as jnp
import numpy as np
import jax.experimental.pallas as pl
import jax.experimental.pallas.tpu as pltpu

F32 = jnp.float32
BF16 = jnp.bfloat16
U32 = jnp.uint32

LANES = 128
LOG2E = float(np.log2(np.e))
LAG = 2
N_EARLY = 10
HEADS_PER_DOT = 1
HEADS_FIRST = 16
FF_TILES = 2
OUT_TILES = 2
DOWN_TILES = 1
FILL = (1, 1, 0)
STAGE_D = 256
STAGE_SLOTS = 6
STAGE_PAD = 16
UP_AT = 2


def _layernorm(x):
    m = jnp.mean(x, axis=-1, keepdims=True)
    c = x - m
    v = jnp.mean(c * c, axis=-1, keepdims=True)
    return c * jax.lax.rsqrt(v + 1e-5)


def _gelu(x):
    return jax.nn.gelu(x, approximate=True)


def _reciprocal(x):
    r = pl.reciprocal(x, approx=True)
    return r * (2.0 - x * r)


def _dot(a, b):
    return jnp.dot(a, b, preferred_element_type=F32)


def _dot_nt(a, b):
    return jax.lax.dot_general(a, b, (((1,), (1,)), ((), ())), preferred_element_type=F32)


def _cat(ref, lo, n, rows=None):
    if ref.dtype == BF16:
        ref = ref.bitcast(U32)
    rows = slice(None) if rows is None else slice(rows.start // 2, rows.stop // 2)
    return jnp.concatenate(
        [pltpu.bitcast(ref[lo + j, rows, :], BF16) for j in range(n)], axis=1)


def _tile(x, j):
    return x[:, j * LANES:(j + 1) * LANES]


def _kernel(x_hbm, mem0_ref, wq_hbm, wk_hbm, wv_hbm, wo_hbm, wg_hbm, wu_hbm, wd_hbm,
            out_hbm,
            x_buf, out_buf, wq, wk, wv, wo, wg, wu, wd, stage,
            h_early, acc_early, qkv_early, h_att, o_att, x1_buf, x2_buf, h_ffn, r_ffn, r_ffn_old, mid, bias2, bias1,
            stage_sem, sems, *, seg, n_seg, n_heads, dh):
    n_mem, dm = mem0_ref.shape
    nd = dm // LANES
    nf = wg.shape[0]
    m2 = 2 * n_mem
    scale = dh ** -0.5

    def seg_rows(s):
        if isinstance(s, int):
            return slice(s * seg, (s + 1) * seg)
        return pl.ds(pl.multiple_of(s * seg, seg), seg)

    def column_copy(src, dst, j, sem):
        cols = slice(j * LANES, (j + 1) * LANES)
        return pltpu.make_async_copy(src.at[:, cols], dst.at[j], sem)

    head_rows = (LAG + 1 + N_EARLY) * seg
    cp_x_head = pltpu.make_async_copy(
        x_hbm.at[0:head_rows], x_buf.at[0:head_rows], sems.at[0])
    cp_x_tail = pltpu.make_async_copy(
        x_hbm.at[head_rows:], x_buf.at[head_rows:], sems.at[1])
    cp_wo = [column_copy(wo_hbm, wo, j, sems.at[2]) for j in range(nd)]

    cp_up = [column_copy(src, dst, j, sems.at[5])
             for j in range(nf) for src, dst in ((wg_hbm, wg), (wu_hbm, wu))]
    cp_down = [column_copy(wd_hbm, wd, j, sems.at[6]) for j in range(nd)]

    n_chunk = dm // STAGE_D
    stage_rows = STAGE_D * n_heads
    srcs = (wq_hbm, wk_hbm, wv_hbm)
    wqkv = (wq, wk, wv)

    def stage_copy(w, c):
        slot = (w * n_chunk + c) % STAGE_SLOTS
        return pltpu.make_async_copy(
            srcs[w].at[pl.ds(pl.multiple_of(c * stage_rows, stage_rows), stage_rows), :],
            stage.at[slot, STAGE_PAD:STAGE_PAD + stage_rows], stage_sem.at[slot])

    def put(ref, rows, x, lo=0):
        for j in range(x.shape[1] // LANES):
            ref[lo + j, rows, :] = _tile(x, j)

    def reset_mem(ref):
        m0 = mem0_ref[...].astype(F32)
        put(ref, slice(0, m2), jnp.concatenate([m0, m0], axis=0).astype(BF16))

    def early_rows(i):
        if isinstance(i, int):
            return slice(m2 + i * seg, m2 + (i + 1) * seg)
        return pl.ds(pl.multiple_of(m2 + i * seg, m2), seg)

    def early_norm(i):
        s = i + LAG if i else 0
        put(h_early, early_rows(i), _layernorm(x_buf[seg_rows(s), :].astype(F32)).astype(BF16))

    stage[:, 0:STAGE_PAD, :] = jnp.zeros((STAGE_SLOTS, STAGE_PAD, dh), BF16)
    stage[:, STAGE_PAD + stage_rows:, :] = jnp.zeros((STAGE_SLOTS, 6 * STAGE_PAD, dh), BF16)
    ahead = STAGE_SLOTS - 1
    cp_x_head.start()
    for i in range(ahead):
        stage_copy(i // n_chunk, i % n_chunk).start()
    reset_mem(h_early)
    acc_early[...] = jnp.zeros_like(acc_early)
    cp_x_head.wait()
    for i in range(N_EARLY + 1):
        early_norm(i)
    stage_u32 = stage.bitcast(U32)
    half = n_heads // 2
    sublane = jax.lax.broadcasted_iota(jnp.int32, (8, dh), 0)

    def gather_rows(slot, base):
        x = {c: stage_u32[slot, pl.ds(base + c, 8, stride=2 * half + 1), :]
             for c in range(-7, half)}
        for k in (1, 2, 4):
            x = {c: jnp.where((sublane & k) != 0, x[c - k], x[c])
                 for c in range(2 * k - 8, half)}
        return [x[j] for j in range(half)]

    for w in range(3):
        def load_chunk(c, carry, w=w):
            nxt = w * n_chunk + c + ahead
            for w2 in range(w, 3):
                @pl.when(nxt // n_chunk == w2)
                def _():
                    stage_copy(w2, nxt - w2 * n_chunk).start()

            if w * n_chunk <= 3 * n_chunk - ahead < (w + 1) * n_chunk:
                @pl.when(nxt == 3 * n_chunk)
                def _():
                    for cp in cp_wo:
                        cp.start()

            if w == 2:
                @pl.when(c == UP_AT)
                def _():
                    for cp in cp_up:
                        cp.start()

            stage_copy(w, c).wait()
            slot = (w * n_chunk + c) % STAGE_SLOTS
            k_tiles = STAGE_D // LANES
            d0 = pl.multiple_of(c * (STAGE_D // 2), STAGE_D // 2)
            for blk in range(STAGE_D // 16):
                base = STAGE_PAD // 2 + blk * 16 * half
                evens = gather_rows(slot, base)
                odds = gather_rows(slot, base + half)
                dst = pl.ds(pl.multiple_of(d0 + blk * 8, 8), 8)
                for j, (ev, od) in enumerate(zip(evens, odds)):
                    wqkv[w][2 * j, dst, :] = (ev & U32(0xFFFF)) | (od << 16)
                    wqkv[w][2 * j + 1, dst, :] = (ev >> 16) | (od & U32(0xFFFF0000))
            for h in range(n_heads):
                y = _dot(_cat(h_early, c * k_tiles, k_tiles),
                         pltpu.bitcast(wqkv[w][h, pl.ds(d0, STAGE_D // 2), :], BF16))
                y = jnp.where(c == 0, y, acc_early[h] + y)
                acc_early[h] = y
                qkv_early[3 * h + w] = y.astype(BF16)
            return carry
        jax.lax.fori_loop(0, n_chunk, load_chunk, 0)

    def make_bias(ref, second_from):
        ri = jax.lax.broadcasted_iota(jnp.int32, ref.shape, 0)
        ci = jax.lax.broadcasted_iota(jnp.int32, ref.shape, 1)

        def second(i):
            return ((i >= n_mem) & (i < m2)) | (i >= second_from)

        visible = (ri < m2) | (ci <= ri)
        ref[...] = jnp.where(second(ri) == second(ci),
                             jnp.where(visible, 0.0, -1e9 / scale), -jnp.inf).astype(F32)

    make_bias(bias2, m2 + seg)
    make_bias(bias1, m2 + seg)

    def ffn_norm():
        put(h_ffn, slice(None), _layernorm(r_ffn[...]).astype(BF16))

    def ffn_up(lo, n):
        hf = _cat(h_ffn, 0, nd)
        y = _gelu(_dot(hf, _cat(wg, lo, n))) * _dot(hf, _cat(wu, lo, n))
        put(mid, slice(None), y.astype(BF16), lo)

    def ffn_down(lo, n, res_ref, store):
        cols = slice(lo * LANES, (lo + n) * LANES)
        store(cols, _dot(_cat(mid, 0, nf), _cat(wd, lo, n)) + res_ref[:, cols])

    def ffn_with(inputs, res_ref, store, norm_next, early=None, before_down=lambda: None):
        down = list(range(0, nd, DOWN_TILES))

        def fill(i):
            for _ in range(FILL[i]):
                ffn_down(down.pop(0), DOWN_TILES, res_ref, store)

        if inputs:
            norm, run = attention(inputs, fill, early=early)
            norm()
        for j in range(0, nf, FF_TILES):
            ffn_up(j, FF_TILES)
        if inputs:
            run()
        if norm_next:
            ffn_norm()
        before_down()
        while down:
            ffn_down(down.pop(0), DOWN_TILES, res_ref, store)

    def attention(inputs, fill=lambda i: None, before_out=lambda: None, early=None):
        n_rows = m2 + len(inputs) * seg
        bias_ref = bias2 if len(inputs) == 2 else bias1

        def norm():
            for i, (load, _, _) in enumerate(inputs):
                if i == 0 and early is not None:
                    continue
                put(h_att, slice(m2 + i * seg, m2 + (i + 1) * seg),
                    _layernorm(load(slice(None))).astype(BF16))

        qkvs, probs = {}, {}

        def project(lo, hi):
            w = jnp.concatenate(
                [_cat(ref, h, 1) for h in range(lo, hi) for ref in wqkv], axis=1)
            if early is None:
                y = _dot(_cat(h_att, 0, nd, slice(0, n_rows)), w).astype(BF16)
            elif len(inputs) == 1:
                y = jnp.concatenate(
                    [qkv_early[j, 0:n_rows, :] for j in range(3 * lo, 3 * hi)], axis=1)
            else:
                lhs = jnp.concatenate([_cat(h_att, 0, nd, slice(0, m2)),
                                       _cat(h_att, 0, nd, slice(m2 + seg, n_rows))], axis=0)
                y = _dot(lhs, w).astype(BF16)
                done = jnp.concatenate(
                    [qkv_early[j, early_rows(early), :] for j in range(3 * lo, 3 * hi)], axis=1)
                y = jnp.concatenate([y[0:m2], done, y[m2:]], axis=0)
            for h in range(lo, hi):
                qkvs[h] = [_tile(y, 3 * (h - lo) + i) for i in range(3)]

        def score(lo, hi):
            for h in range(lo, hi):
                bias = bias_ref[...]
                s = jnp.where(bias == 0.0, _dot_nt(qkvs[h][0], qkvs[h][1]), bias)
                p = jnp.exp2((s - jnp.max(s, axis=-1, keepdims=True)) * (scale * LOG2E))
                probs[h] = (p.astype(BF16), _reciprocal(jnp.sum(p, axis=-1, keepdims=True)))

        def mix(lo, hi):
            for h in range(lo, hi):
                p, inv = probs.pop(h)
                o_att[h, 0:n_rows, :] = (_dot(p, qkvs.pop(h)[2]) * inv).astype(BF16)

        def project_out(lo, n):
            cols = slice(lo * LANES, (lo + n) * LANES)
            y = _dot(_cat(o_att, 0, n_heads, slice(0, n_rows)), _cat(wo, lo, n))
            mem = y[0:m2]
            if len(inputs) == 1:
                keep = jnp.concatenate(
                    [h_att[j, 0:m2, :] for j in range(lo, lo + n)], axis=1).astype(F32)
                row = jax.lax.broadcasted_iota(jnp.int32, mem.shape, 0)
                mem = jnp.where(row // n_mem == inputs[0][2], mem, keep)
            put(h_att, slice(0, m2), mem.astype(BF16), lo)
            for i, (load, slot, _) in enumerate(inputs):
                slot(cols, load(cols) + y[m2 + i * seg:m2 + (i + 1) * seg])

        def run():
            g = HEADS_FIRST if early is not None and len(inputs) == 1 else HEADS_PER_DOT
            n_grp = n_heads // g
            for i in range(n_grp + 2):
                if i < n_grp:
                    project(i * g, (i + 1) * g)
                else:
                    fill(i - n_grp)
                if 0 <= i - 2:
                    mix((i - 2) * g, (i - 1) * g)
                if 0 <= i - 1 < n_grp:
                    score((i - 1) * g, i * g)
            fill(2)
            before_out()
            for j in range(0, nd, OUT_TILES):
                project_out(j, OUT_TILES)

        return norm, run

    def load_x(s):
        return lambda cols: x_buf[seg_rows(s), cols].astype(F32)

    def load_x2(s):
        return lambda cols: x2_buf[seg_rows(s % 2), cols]

    def to_ffn(slot, ref=r_ffn):
        def store(cols, y):
            ref[seg_rows(slot), cols] = y
        return store

    def store_step(s_x2, s_out):
        def store(cols, y):
            x2_buf[seg_rows(s_x2 % 2), cols] = y[0:seg]
            out_buf[seg_rows(s_out), cols] = y[seg:].astype(BF16)
        return store

    def wait_wo():
        for cp in cp_wo:
            cp.wait()

    reset_mem(h_att)
    _, run = attention([(load_x(0), to_ffn(0, x1_buf), 0)], before_out=wait_wo, early=0)
    run()

    for cp in cp_down:
        cp.start()
    def first_layer_only(s, carry):
        norm, run = attention([(load_x(s), to_ffn(s, x1_buf), 0)])
        norm()
        run()
        return carry

    jax.lax.fori_loop(1, LAG + 1, first_layer_only, 0)

    def store_x2(cols, y):
        x2_buf[:, cols] = y

    def wait_down():
        for cp in cp_down:
            cp.wait()

    r_ffn[...] = x1_buf[0:2 * seg, :]
    ffn_norm()
    for cp in cp_up:
        cp.wait()
    ffn_with([], r_ffn, store_x2, False, before_down=wait_down)
    cp_x_tail.start()
    r_ffn[0:seg, :] = x1_buf[2 * seg:, :]
    make_bias(bias1, m2)
    norm, run = attention([(load_x2(0), to_ffn(1), 1)])
    norm()
    run()
    ffn_norm()

    def step(t, carry, early=False):
        r_ffn_old[...] = r_ffn[...]
        ffn_with([(load_x(t), to_ffn(0), 0), (load_x2(t - 2), to_ffn(1), 1)],
                 r_ffn_old, store_step(t - 1, t - 3), True, t - LAG if early else None)
        return carry

    first_full = LAG + 1 + N_EARLY
    jax.lax.fori_loop(LAG + 1, first_full, functools.partial(step, early=True), 0)
    cp_x_tail.wait()
    jax.lax.fori_loop(first_full, n_seg, step, 0)

    done = (n_seg - 3) * seg
    cp_out_head = pltpu.make_async_copy(out_buf.at[0:done], out_hbm.at[0:done], sems.at[3])
    cp_out_tail = pltpu.make_async_copy(out_buf.at[done:], out_hbm.at[done:], sems.at[4])
    cp_out_head.start()
    r_ffn_old[...] = r_ffn[...]
    ffn_with([(load_x2(n_seg - 2), to_ffn(0), 1)],
             r_ffn_old, store_step(n_seg - 1, n_seg - 3), False)
    norm, run = attention([(load_x2(n_seg - 1), to_ffn(1), 1)])
    norm()
    run()
    ffn_norm()

    def store_out(cols, y):
        out_buf[(n_seg - 2) * seg:, cols] = y.astype(BF16)

    ffn_with([], r_ffn, store_out, False)
    cp_out_tail.start()
    cp_out_head.wait()
    cp_out_tail.wait()


@functools.partial(jax.jit, static_argnames=("A_seg_len",))
def pallas_interleave_layers__memory_aug_recurrent_mem_tr__glu_gated_geglu__prompt_kernel(
    A_x: jax.Array,
    A_mem0: jax.Array,
    A_Wq: jax.Array,
    A_Wk: jax.Array,
    A_Wv: jax.Array,
    A_Wo: jax.Array,
    A_seg_len: int,
    B_x: jax.Array,
    B_w_gate: jax.Array,
    B_w_up: jax.Array,
    B_w_down: jax.Array,
):
    del B_x
    batch, s, dm = A_x.shape
    assert batch == 1
    _, n_heads, dh = A_Wq.shape
    n_mem = A_mem0.shape[1]
    dff = B_w_gate.shape[1]
    seg = int(A_seg_len)
    n_seg = s // seg
    rows = 2 * (n_mem + seg)
    early = 2 * n_mem + (1 + N_EARLY) * seg
    nd, nf = dm // LANES, dff // LANES
    assert dh == LANES

    hbm = pl.BlockSpec(memory_space=pl.ANY)
    out = pl.pallas_call(
        functools.partial(_kernel, seg=seg, n_seg=n_seg, n_heads=n_heads, dh=dh),
        out_shape=jax.ShapeDtypeStruct((s, dm), A_x.dtype),
        in_specs=[hbm, pl.BlockSpec(memory_space=pltpu.VMEM)] + [hbm] * 7,
        out_specs=hbm,
        scratch_shapes=[
            pltpu.VMEM((s, dm), BF16),
            pltpu.VMEM((s, dm), BF16),
            pltpu.VMEM((n_heads, dm // 2, dh), U32),
            pltpu.VMEM((n_heads, dm // 2, dh), U32),
            pltpu.VMEM((n_heads, dm // 2, dh), U32),
            pltpu.VMEM((nd, n_heads * dh, LANES), BF16),
            pltpu.VMEM((nf, dm, LANES), BF16),
            pltpu.VMEM((nf, dm, LANES), BF16),
            pltpu.VMEM((nd, dff, LANES), BF16),
            pltpu.VMEM((STAGE_SLOTS, STAGE_D * n_heads + 7 * STAGE_PAD, dh), BF16),
            pltpu.VMEM((nd, early, LANES), BF16),
            pltpu.VMEM((n_heads, early, dh), F32),
            pltpu.VMEM((3 * n_heads, early, dh), BF16),
            pltpu.VMEM((nd, rows, LANES), BF16),
            pltpu.VMEM((n_heads, rows, dh), BF16),
            pltpu.VMEM((3 * seg, dm), F32),
            pltpu.VMEM((2 * seg, dm), F32),
            pltpu.VMEM((nd, 2 * seg, LANES), BF16),
            pltpu.VMEM((2 * seg, dm), F32),
            pltpu.VMEM((2 * seg, dm), F32),
            pltpu.VMEM((nf, 2 * seg, LANES), BF16),
            pltpu.VMEM((rows, rows), F32),
            pltpu.VMEM((rows - seg, rows - seg), F32),
            pltpu.SemaphoreType.DMA((STAGE_SLOTS,)),
            pltpu.SemaphoreType.DMA((7,)),
        ],
        compiler_params=pltpu.CompilerParams(vmem_limit_bytes=112 * 2**20),
    )(
        A_x.reshape(s, dm),
        A_mem0.reshape(n_mem, dm),
        A_Wq.reshape(dm * n_heads, dh),
        A_Wk.reshape(dm * n_heads, dh),
        A_Wv.reshape(dm * n_heads, dh),
        A_Wo.reshape(n_heads * dh, dm),
        B_w_gate,
        B_w_up,
        B_w_down,
    )
    return out.reshape(A_x.shape)
```

```python
import functools

import jax
import jax.numpy as jnp
import numpy as np
import jax.experimental.pallas as pl
import jax.experimental.pallas.tpu as pltpu

F32 = jnp.float32
BF16 = jnp.bfloat16
U32 = jnp.uint32

_approx_reciprocal = pltpu.reciprocal if hasattr(pltpu, "reciprocal") else pl.reciprocal

LANES = 128
LOG2E = float(np.log2(np.e))
LAG = 2
N_EARLY = 12
HEADS_PER_DOT = 1
HEADS_FIRST = 16
FF_TILES = 2
OUT_TILES = 2
DOWN_TILES = 1
FILL = (1, 1, 0)
STAGE_D = 256
STAGE_SLOTS = 8
STAGE_PAD = 16
UP_AT = 0


def _layernorm(x):
    m = jnp.mean(x, axis=-1, keepdims=True)
    c = x - m
    v = jnp.mean(c * c, axis=-1, keepdims=True)
    return c * jax.lax.rsqrt(v + 1e-5)


def _gelu(x):
    return jax.nn.gelu(x, approximate=True)


def _reciprocal(x):
    r = _approx_reciprocal(x, approx=True)
    return r * (2.0 - x * r)


def _dot(a, b):
    return jnp.dot(a, b, preferred_element_type=F32)


def _dot_nt(a, b):
    return jax.lax.dot_general(a, b, (((1,), (1,)), ((), ())), preferred_element_type=F32)


def _cat(ref, lo, n, rows=None):
    if ref.dtype == BF16:
        ref = ref.bitcast(U32)
    rows = slice(None) if rows is None else slice(rows.start // 2, rows.stop // 2)
    return jnp.concatenate(
        [pltpu.bitcast(ref[lo + j, rows, :], BF16) for j in range(n)], axis=1)


def _tile(x, j):
    return x[:, j * LANES:(j + 1) * LANES]


def _kernel(x_hbm, mem0_ref, wq_hbm, wk_hbm, wv_hbm, wo_hbm, wg_hbm, wu_hbm, wd_hbm,
            out_hbm,
            x_buf, out_buf, wq, wk, wv, wo, wg, wu, wd, stage,
            h_early, acc_early, qkv_early, h_att, o_att, x2_buf, h_ffn, r_ffn, r_ffn_old, mid, bias2, bias1,
            stage_sem, sems, *, seg, n_seg, n_heads, dh):
    n_mem, dm = mem0_ref.shape
    nd = dm // LANES
    nf = wg.shape[0]
    m2 = 2 * n_mem
    scale = dh ** -0.5

    def seg_rows(s):
        if isinstance(s, int):
            return slice(s * seg, (s + 1) * seg)
        return pl.ds(pl.multiple_of(s * seg, seg), seg)

    def column_copy(src, dst, j, sem):
        cols = slice(j * LANES, (j + 1) * LANES)
        return pltpu.make_async_copy(src.at[:, cols], dst.at[j], sem)

    first_full = LAG + N_EARLY
    head_rows = first_full * seg
    cp_x_head = pltpu.make_async_copy(
        x_hbm.at[0:head_rows], x_buf.at[0:head_rows], sems.at[0])
    cp_x_tail = pltpu.make_async_copy(
        x_hbm.at[head_rows:], x_buf.at[head_rows:], sems.at[1])
    cp_wo = [column_copy(wo_hbm, wo, j, sems.at[2]) for j in range(nd)]
    cp_up = [column_copy(src, dst, j, sems.at[5])
             for j in range(nf) for src, dst in ((wg_hbm, wg), (wu_hbm, wu))]
    cp_down = [column_copy(wd_hbm, wd, j, sems.at[6]) for j in range(nd)]

    n_chunk = dm // STAGE_D
    stage_rows = STAGE_D * n_heads
    srcs = (wq_hbm, wk_hbm, wv_hbm)
    wqkv = (wq, wk, wv)

    def stage_copy(w, c):
        slot = (w * n_chunk + c) % STAGE_SLOTS
        return pltpu.make_async_copy(
            srcs[w].at[pl.ds(pl.multiple_of(c * stage_rows, stage_rows), stage_rows), :],
            stage.at[slot, STAGE_PAD:STAGE_PAD + stage_rows], stage_sem.at[slot])

    def put(ref, rows, x, lo=0):
        for j in range(x.shape[1] // LANES):
            ref[lo + j, rows, :] = _tile(x, j)

    def reset_mem(ref):
        m0 = mem0_ref[...].astype(F32)
        put(ref, slice(0, m2), jnp.concatenate([m0, m0], axis=0).astype(BF16))

    def early_rows(i):
        if isinstance(i, int):
            return slice(m2 + i * seg, m2 + (i + 1) * seg)
        return pl.ds(pl.multiple_of(m2 + i * seg, m2), seg)

    def early_norm(i):
        s = i + LAG - 1 if i else 0
        put(h_early, early_rows(i), _layernorm(x_buf[seg_rows(s), :].astype(F32)).astype(BF16))
    stage[:, 0:STAGE_PAD, :] = jnp.zeros((STAGE_SLOTS, STAGE_PAD, dh), BF16)
    stage[:, STAGE_PAD + stage_rows:, :] = jnp.zeros((STAGE_SLOTS, 6 * STAGE_PAD, dh), BF16)
    ahead = STAGE_SLOTS - 1
    cp_x_head.start()
    for i in range(ahead):
        stage_copy(i // n_chunk, i % n_chunk).start()
    reset_mem(h_early)
    acc_early[...] = jnp.zeros_like(acc_early)
    cp_x_head.wait()
    for i in range(N_EARLY + 1):
        early_norm(i)
    stage_u32 = stage.bitcast(U32)
    half = n_heads // 2
    sublane = jax.lax.broadcasted_iota(jnp.int32, (8, dh), 0)

    def gather_rows(slot, base):
        x = {c: stage_u32[slot, pl.ds(base + c, 8, stride=2 * half + 1), :]
             for c in range(-7, half)}
        for k in (1, 2, 4):
            x = {c: jnp.where((sublane & k) != 0, x[c - k], x[c])
                 for c in range(2 * k - 8, half)}
        return [x[j] for j in range(half)]

    for w in range(3):
        def load_chunk(c, carry, w=w):
            nxt = w * n_chunk + c + ahead
            for w2 in range(w, 3):
                @pl.when(nxt // n_chunk == w2)
                def _():
                    stage_copy(w2, nxt - w2 * n_chunk).start()

            if w * n_chunk <= 3 * n_chunk - ahead < (w + 1) * n_chunk:
                @pl.when(nxt == 3 * n_chunk)
                def _():
                    for cp in cp_wo:
                        cp.start()

            if w == 2:
                @pl.when(c == UP_AT)
                def _():
                    for cp in cp_up:
                        cp.start()

            stage_copy(w, c).wait()
            slot = (w * n_chunk + c) % STAGE_SLOTS
            k_tiles = STAGE_D // LANES
            d0 = pl.multiple_of(c * (STAGE_D // 2), STAGE_D // 2)
            for blk in range(STAGE_D // 16):
                base = STAGE_PAD // 2 + blk * 16 * half
                evens = gather_rows(slot, base)
                odds = gather_rows(slot, base + half)
                dst = pl.ds(pl.multiple_of(d0 + blk * 8, 8), 8)
                for j, (ev, od) in enumerate(zip(evens, odds)):
                    wqkv[w][2 * j, dst, :] = (ev & U32(0xFFFF)) | (od << 16)
                    wqkv[w][2 * j + 1, dst, :] = (ev >> 16) | (od & U32(0xFFFF0000))
            for h in range(n_heads):
                y = _dot(_cat(h_early, c * k_tiles, k_tiles),
                         pltpu.bitcast(wqkv[w][h, pl.ds(d0, STAGE_D // 2), :], BF16))
                y = jnp.where(c == 0, y, acc_early[h] + y)
                acc_early[h] = y
                qkv_early[3 * h + w] = y.astype(BF16)
            return carry
        jax.lax.fori_loop(0, n_chunk, load_chunk, 0)

    def make_bias(ref, second_from):
        ri = jax.lax.broadcasted_iota(jnp.int32, ref.shape, 0)
        ci = jax.lax.broadcasted_iota(jnp.int32, ref.shape, 1)

        def second(i):
            return ((i >= n_mem) & (i < m2)) | (i >= second_from)

        visible = (ri < m2) | (ci <= ri)
        ref[...] = jnp.where(second(ri) == second(ci),
                             jnp.where(visible, 0.0, -1e9 / scale), -jnp.inf).astype(F32)

    make_bias(bias2, m2 + seg)
    make_bias(bias1, m2 + seg)

    def ffn_norm():
        put(h_ffn, slice(None), _layernorm(r_ffn[...]).astype(BF16))

    def ffn_up(lo, n):
        hf = _cat(h_ffn, 0, nd)
        y = _gelu(_dot(hf, _cat(wg, lo, n))) * _dot(hf, _cat(wu, lo, n))
        put(mid, slice(None), y.astype(BF16), lo)

    def ffn_down(lo, n, res_ref, store):
        cols = slice(lo * LANES, (lo + n) * LANES)
        store(cols, _dot(_cat(mid, 0, nf), _cat(wd, lo, n)) + res_ref[:, cols])

    def ffn_with(inputs, res_ref, store, norm_next, early=None, before_down=lambda: None):
        down = list(range(0, nd, DOWN_TILES))

        def fill(i):
            for _ in range(FILL[i]):
                ffn_down(down.pop(0), DOWN_TILES, res_ref, store)

        if inputs:
            norm, run = attention(inputs, fill, early=early)
            norm()
        for j in range(0, nf, FF_TILES):
            ffn_up(j, FF_TILES)
        if inputs:
            run()
        if norm_next:
            ffn_norm()
        before_down()
        while down:
            ffn_down(down.pop(0), DOWN_TILES, res_ref, store)

    def attention(inputs, fill=lambda i: None, before_out=lambda: None, early=None):
        n_rows = m2 + len(inputs) * seg
        bias_ref = bias2 if len(inputs) == 2 else bias1

        def norm():
            for i, (load, _, _) in enumerate(inputs):
                if i == 0 and early is not None:
                    continue
                put(h_att, slice(m2 + i * seg, m2 + (i + 1) * seg),
                    _layernorm(load(slice(None))).astype(BF16))

        qkvs, probs = {}, {}

        def project(lo, hi):
            w = jnp.concatenate(
                [_cat(ref, h, 1) for h in range(lo, hi) for ref in wqkv], axis=1)
            if early is None:
                y = _dot(_cat(h_att, 0, nd, slice(0, n_rows)), w).astype(BF16)
            elif len(inputs) == 1:
                y = jnp.concatenate(
                    [qkv_early[j, 0:n_rows, :] for j in range(3 * lo, 3 * hi)], axis=1)
            else:
                lhs = jnp.concatenate([_cat(h_att, 0, nd, slice(0, m2)),
                                       _cat(h_att, 0, nd, slice(m2 + seg, n_rows))], axis=0)
                y = _dot(lhs, w).astype(BF16)
                done = jnp.concatenate(
                    [qkv_early[j, early_rows(early), :] for j in range(3 * lo, 3 * hi)], axis=1)
                y = jnp.concatenate([y[0:m2], done, y[m2:]], axis=0)
            for h in range(lo, hi):
                qkvs[h] = [_tile(y, 3 * (h - lo) + i) for i in range(3)]

        def score(lo, hi):
            for h in range(lo, hi):
                bias = bias_ref[...]
                s = jnp.where(bias == 0.0, _dot_nt(qkvs[h][0], qkvs[h][1]), bias)
                p = jnp.exp2((s - jnp.max(s, axis=-1, keepdims=True)) * (scale * LOG2E))
                probs[h] = (p.astype(BF16), _reciprocal(jnp.sum(p, axis=-1, keepdims=True)))

        def mix(lo, hi):
            for h in range(lo, hi):
                p, inv = probs.pop(h)
                o_att[h, 0:n_rows, :] = (_dot(p, qkvs.pop(h)[2]) * inv).astype(BF16)

        def project_out(lo, n):
            cols = slice(lo * LANES, (lo + n) * LANES)
            y = _dot(_cat(o_att, 0, n_heads, slice(0, n_rows)), _cat(wo, lo, n))
            mem = y[0:m2]
            if len(inputs) == 1:
                keep = jnp.concatenate(
                    [h_att[j, 0:m2, :] for j in range(lo, lo + n)], axis=1).astype(F32)
                row = jax.lax.broadcasted_iota(jnp.int32, mem.shape, 0)
                mem = jnp.where(row // n_mem == inputs[0][2], mem, keep)
            put(h_att, slice(0, m2), mem.astype(BF16), lo)
            for i, (load, slot, _) in enumerate(inputs):
                slot(cols, load(cols) + y[m2 + i * seg:m2 + (i + 1) * seg])

        def run():
            g = HEADS_FIRST if early is not None and len(inputs) == 1 else HEADS_PER_DOT
            n_grp = n_heads // g
            for i in range(n_grp + 2):
                if i < n_grp:
                    project(i * g, (i + 1) * g)
                else:
                    fill(i - n_grp)
                if 0 <= i - 2:
                    mix((i - 2) * g, (i - 1) * g)
                if 0 <= i - 1 < n_grp:
                    score((i - 1) * g, i * g)
            fill(2)
            before_out()
            for j in range(0, nd, OUT_TILES):
                project_out(j, OUT_TILES)

        return norm, run

    def load_x(s):
        return lambda cols: x_buf[seg_rows(s), cols].astype(F32)

    def load_x2(s):
        return lambda cols: x2_buf[seg_rows(s % 2), cols]

    def to_ffn(slot):
        def store(cols, y):
            r_ffn[seg_rows(slot), cols] = y
        return store

    def store_step(s_x2, s_out):
        def store(cols, y):
            x2_buf[seg_rows(s_x2 % 2), cols] = y[0:seg]
            out_buf[seg_rows(s_out), cols] = y[seg:].astype(BF16)
        return store

    def wait_wo():
        for cp in cp_wo:
            cp.wait()

    reset_mem(h_att)
    _, run = attention([(load_x(0), to_ffn(0), 0)], before_out=wait_wo, early=0)
    run()
    for cp in cp_down:
        cp.start()
    norm, run = attention([(load_x(1), to_ffn(1), 0)])
    norm()
    run()

    def store_x2(cols, y):
        x2_buf[:, cols] = y

    def wait_down():
        for cp in cp_down:
            cp.wait()
    ffn_norm()
    for cp in cp_up:
        cp.wait()
    ffn_with([], r_ffn, store_x2, False, before_down=wait_down)
    cp_x_tail.start()
    norm, run = attention([(load_x(2), to_ffn(0), 0), (load_x2(0), to_ffn(1), 1)], early=1)
    norm()
    run()
    ffn_norm()

    def step(t, carry, early=False):
        r_ffn_old[...] = r_ffn[...]
        ffn_with([(load_x(t), to_ffn(0), 0), (load_x2(t - 2), to_ffn(1), 1)],
                 r_ffn_old, store_step(t - 1, t - 3), True, t - 1 if early else None)
        return carry
    jax.lax.fori_loop(LAG + 1, first_full, functools.partial(step, early=True), 0)
    cp_x_tail.wait()
    jax.lax.fori_loop(first_full, n_seg, step, 0)

    done = (n_seg - 3) * seg
    cp_out_head = pltpu.make_async_copy(out_buf.at[0:done], out_hbm.at[0:done], sems.at[3])
    cp_out_tail = pltpu.make_async_copy(out_buf.at[done:], out_hbm.at[done:], sems.at[4])
    cp_out_head.start()
    make_bias(bias1, m2)
    r_ffn_old[...] = r_ffn[...]
    ffn_with([(load_x2(n_seg - 2), to_ffn(0), 1)],
             r_ffn_old, store_step(n_seg - 1, n_seg - 3), False)
    norm, run = attention([(load_x2(n_seg - 1), to_ffn(1), 1)])
    norm()
    run()
    ffn_norm()

    def store_out(cols, y):
        out_buf[(n_seg - 2) * seg:, cols] = y.astype(BF16)
    ffn_with([], r_ffn, store_out, False)
    cp_out_tail.start()
    cp_out_head.wait()
    cp_out_tail.wait()


@functools.partial(jax.jit, static_argnames=("A_seg_len",))
def pallas_interleave_layers__memory_aug_recurrent_mem_tr__glu_gated_geglu__prompt_kernel(
    A_x: jax.Array,
    A_mem0: jax.Array,
    A_Wq: jax.Array,
    A_Wk: jax.Array,
    A_Wv: jax.Array,
    A_Wo: jax.Array,
    A_seg_len: int,
    B_x: jax.Array,
    B_w_gate: jax.Array,
    B_w_up: jax.Array,
    B_w_down: jax.Array,
):
    del B_x
    batch, s, dm = A_x.shape
    assert batch == 1
    _, n_heads, dh = A_Wq.shape
    n_mem = A_mem0.shape[1]
    dff = B_w_gate.shape[1]
    seg = int(A_seg_len)
    n_seg = s // seg
    rows = 2 * (n_mem + seg)
    early = 2 * n_mem + (1 + N_EARLY) * seg
    nd, nf = dm // LANES, dff // LANES
    assert dh == LANES

    hbm = pl.BlockSpec(memory_space=pl.ANY)
    out = pl.pallas_call(
        functools.partial(_kernel, seg=seg, n_seg=n_seg, n_heads=n_heads, dh=dh),
        out_shape=jax.ShapeDtypeStruct((s, dm), A_x.dtype),
        in_specs=[hbm, pl.BlockSpec(memory_space=pltpu.VMEM)] + [hbm] * 7,
        out_specs=hbm,
        scratch_shapes=[
            pltpu.VMEM((s, dm), BF16),
            pltpu.VMEM((s, dm), BF16),
            pltpu.VMEM((n_heads, dm // 2, dh), U32),
            pltpu.VMEM((n_heads, dm // 2, dh), U32),
            pltpu.VMEM((n_heads, dm // 2, dh), U32),
            pltpu.VMEM((nd, n_heads * dh, LANES), BF16),
            pltpu.VMEM((nf, dm, LANES), BF16),
            pltpu.VMEM((nf, dm, LANES), BF16),
            pltpu.VMEM((nd, dff, LANES), BF16),
            pltpu.VMEM((STAGE_SLOTS, STAGE_D * n_heads + 7 * STAGE_PAD, dh), BF16),
            pltpu.VMEM((nd, early, LANES), BF16),
            pltpu.VMEM((n_heads, early, dh), F32),
            pltpu.VMEM((3 * n_heads, early, dh), BF16),
            pltpu.VMEM((nd, rows, LANES), BF16),
            pltpu.VMEM((n_heads, rows, dh), BF16),
            pltpu.VMEM((2 * seg, dm), F32),
            pltpu.VMEM((nd, 2 * seg, LANES), BF16),
            pltpu.VMEM((2 * seg, dm), F32),
            pltpu.VMEM((2 * seg, dm), F32),
            pltpu.VMEM((nf, 2 * seg, LANES), BF16),
            pltpu.VMEM((rows, rows), F32),
            pltpu.VMEM((rows - seg, rows - seg), F32),
            pltpu.SemaphoreType.DMA((STAGE_SLOTS,)),
            pltpu.SemaphoreType.DMA((7,)),
        ],
        compiler_params=pltpu.CompilerParams(vmem_limit_bytes=112 * 2**20),
    )(
        A_x.reshape(s, dm),
        A_mem0.reshape(n_mem, dm),
        A_Wq.reshape(dm * n_heads, dh),
        A_Wk.reshape(dm * n_heads, dh),
        A_Wv.reshape(dm * n_heads, dh),
        A_Wo.reshape(n_heads * dh, dm),
        B_w_gate,
        B_w_up,
        B_w_down,
    )
    return out.reshape(A_x.shape)
```
